```python
import jax
import jax.numpy as jnp

def _softmax(x, axis=-1):
    return jax.nn.softmax(x, axis=axis)

def _gelu(x):
    return jax.nn.gelu(x, approximate=True)

def _silu(x):
    return jax.nn.silu(x)

def _sigmoid(x):
    return jax.nn.sigmoid(x)

def _layernorm(x, axis=-1, eps=1e-05):
    m = jnp.mean(x, axis=axis, keepdims=True)
    v = jnp.var(x, axis=axis, keepdims=True)
    return (x - m) / jnp.sqrt(v + eps)

def _scatter_add(tgt, idx, src, axis=0):
    return tgt.at[idx].add(src)

def _segment_sum(src, seg, n):
    return jax.ops.segment_sum(src, seg, n)

class _Rng:

    def __init__(self, key):
        self._k = key

    def _next(self):
        self._k, sub = jax.random.split(self._k)
        return sub

    def normal(self, shape):
        return jax.random.normal(self._next(), shape, dtype=jnp.bfloat16)

    def randint(self, lo, hi, shape):
        return jax.random.randint(self._next(), shape, lo, hi, dtype=jnp.int32)

    def uniform(self, shape, lo=0.0, hi=1.0):
        return jax.random.uniform(self._next(), shape, jnp.bfloat16, lo, hi)

    def permutation(self, n):
        return jax.random.permutation(self._next(), n)
kernel_name = 'parallel_sum__memory_aug_infini_attn__moe_arch_mod__prompt'

def setup_inputs():
    _rng = _Rng(jax.random.key(int.from_bytes(__import__("os").urandom(4), "little")))
    _w = lambda a: (lambda t: t.astype(jnp.bfloat16) if jnp.issubdtype(t.dtype, jnp.floating) else t)(jnp.asarray(a))

    def _A_setup():
        B, S, D, H = (1, 2048, 576, 32)
        N = 4
        L = max(1, S // N)
        sc = D ** (-0.5)
        return {'x': _w((lambda *s: _rng.normal(s) * 0.05)(B, N * L, D)), 'wq': _w((lambda *s: _rng.normal(s) * 0.05)(D, D) * sc), 'wk': _w((lambda *s: _rng.normal(s) * 0.05)(D, D) * sc), 'wv': _w((lambda *s: _rng.normal(s) * 0.05)(D, D) * sc), 'wo': _w((lambda *s: _rng.normal(s) * 0.05)(D, D) * sc), 'beta': _w((lambda *s: _rng.normal(s) * 0.05)(H))}
    _A_in = _A_setup()

    def _B_setup():
        B, S, D, F, C = (1, 2048, 576, 4608, 2)
        return {'x': _w((lambda *s: _rng.normal(s) * 0.05)(B, S, D)), 'w_r': _w((lambda *s: _rng.normal(s) * 0.05)(D)), 'w_gate': _w((lambda *s: _rng.normal(s) * 0.05)(D, F)), 'w_up': _w((lambda *s: _rng.normal(s) * 0.05)(D, F)), 'w_down': _w((lambda *s: _rng.normal(s) * 0.05)(F, D))}
    _B_in = _B_setup()
    return {'A_x': _A_in['x'], 'A_wq': _A_in['wq'], 'A_wk': _A_in['wk'], 'A_wv': _A_in['wv'], 'A_wo': _A_in['wo'], 'A_beta': _A_in['beta'], 'B_x': _B_in['x'], 'B_w_r': _B_in['w_r'], 'B_w_gate': _B_in['w_gate'], 'B_w_up': _B_in['w_up'], 'B_w_down': _B_in['w_down']}

def reference(A_x, A_wq, A_wk, A_wv, A_wo, A_beta, B_x, B_w_r, B_w_gate, B_w_up, B_w_down):

    def _A_ref(x, wq, wk, wv, wo, beta):
        B, S, D = x.shape
        H = 32
        Dh = D // H
        N = 4
        L = S // N
        q = (lambda x, *d: x.transpose(*d))((x @ wq).reshape(B, S, H, Dh), 0, 2, 1, 3).reshape(B, H, N, L, Dh)
        k = (lambda x, *d: x.transpose(*d))((x @ wk).reshape(B, S, H, Dh), 0, 2, 1, 3).reshape(B, H, N, L, Dh)
        v = (lambda x, *d: x.transpose(*d))((x @ wv).reshape(B, S, H, Dh), 0, 2, 1, 3).reshape(B, H, N, L, Dh)
        phi = lambda t: jnp.where(t > 0, t + 1.0, jnp.exp(t))
        scale = Dh ** (-0.5)
        ar = jnp.arange(L)
        mask = (lambda x, dt: x.astype(dt))(ar[:, None] < ar[None, :], x.dtype) * -1000000000.0
        g = _sigmoid(beta).reshape(1, H, 1, 1)
        M = jnp.einsum('bhd,bhe->bhde', q[:, :, 0, 0, :] * 0.0, q[:, :, 0, 0, :] * 0.0)
        z = q[:, :, 0, 0, :] * 0.0
        outs = []
        for s in range(N):
            qs, ks, vs = (q[:, :, s].copy(), k[:, :, s].copy(), v[:, :, s].copy())
            logits = jnp.einsum('bhqd,bhkd->bhqk', qs, ks) * scale + mask
            p = _softmax(logits, axis=-1)
            a_dot = jnp.einsum('bhqk,bhkd->bhqd', p, vs)
            pq = phi(qs)
            num = jnp.einsum('bhld,bhde->bhle', pq, M)
            den = jnp.einsum('bhld,bhd->bhl', pq, z)[..., None] + 1e-06
            a_mem = num / den
            o = g * a_mem + (1.0 - g) * a_dot
            outs.append(o)
            pk = phi(ks)
            M = M + jnp.einsum('bhld,bhle->bhde', pk, vs)
            z = z + jnp.einsum('bhld->bhd', pk)
        o = (lambda x, *d: x.transpose(*d))(jnp.stack(outs, 2).reshape(B, H, S, Dh), 0, 2, 1, 3).reshape(B, S, D)
        return o @ wo

    def _B_ref(x, w_r, w_gate, w_up, w_down):
        B, S, D = x.shape
        C = 2
        r = x @ w_r
        idx = jnp.argsort(-r, axis=-1)[:, :C]
        idx_e = jnp.repeat(idx.reshape(B, C, 1), D, axis=2)
        x_sel = jnp.take_along_axis(x, idx_e, axis=1)
        g = _silu(x_sel @ w_gate)
        u = x_sel @ w_up
        y = g * u @ w_down
        r_sel = _sigmoid(jnp.take_along_axis(r, idx, axis=1))
        y = y * r_sel.reshape(B, C, 1)
        b_off = (jnp.arange(B) * S).reshape(B, 1)
        flat_idx = (idx + b_off).reshape(B * C)
        zero = (x * 0.0).reshape(B * S, D)
        upd = _scatter_add(zero, flat_idx, y.reshape(B * C, D), axis=0)
        return x + upd.reshape(B, S, D)
    x = A_x
    xn = _layernorm(x, axis=-1)
    return x + _A_ref(xn, A_wq, A_wk, A_wv, A_wo, A_beta) + _B_ref(xn, B_w_r, B_w_gate, B_w_up, B_w_down)
```

```python
import jax
import jax.numpy as jnp
import numpy as np
from jax import lax
import jax.experimental.pallas as pl
import jax.experimental.pallas.tpu as pltpu

F32, BF16, U32 = jnp.float32, jnp.bfloat16, jnp.uint32

S, D, H, NSEG, FF = 2048, 576, 32, 4, 4608
DH = D // H
L = S // NSEG
T = 128
NT = L // T
NG = H // 4
GW = 80
DE = D + 16
FC = FF // NSEG
QSCALE = float(DH ** -0.5 * np.log2(np.e))
EPS = float(np.asarray(1e-5, dtype=jnp.bfloat16))
NEG = -1e30
CHUNKS = ((0, 128), (128, 256), (256, 384), (384, 512), (512, 576))
PV_DELAY = 2


def _dot(a, b, ca=1, cb=0):
    return lax.dot_general(a, b, (((ca,), (cb,)), ((), ())), preferred_element_type=F32)


def _iota(shape, dim):
    return lax.broadcasted_iota(jnp.int32, shape, dim)


def _round(x):
    return x.astype(BF16).astype(F32)


def _phi(t):
    return jnp.where(t > 0, t + 1.0, jnp.exp(t))


def _win(g):
    return (72 * g // 16) * 16


def _kernel(x_hbm, wq_hbm, wk_hbm, wv_hbm, wo_hbm, beta_hbm, wr_hbm, wg_hbm, wu_hbm, wd_hbm,
            out_hbm,
            xs, xn, wq, wk, wv, wo, beta, wr, wg, wu, wd,
            qt, pq, vt, kt, kg, ot, rr, wrb, gate, mask, outb,
            sem_x, sem_w, sem_f, sem_o):
    def x_copy(s):
        return pltpu.make_async_copy(
            x_hbm.at[:, pl.ds(pl.multiple_of(s * L, L), L)], xs.at[s], sem_x.at[s])

    def out_copy(s):
        return pltpu.make_async_copy(
            outb.at[s], out_hbm.at[:, pl.ds(pl.multiple_of(s * L, L), L)], sem_o.at[s])

    c_wr = pltpu.make_async_copy(wr_hbm, wr, sem_w.at[0])
    c_beta = pltpu.make_async_copy(beta_hbm, beta, sem_w.at[1])
    c_wq = pltpu.make_async_copy(wq_hbm, wq, sem_w.at[2])
    c_wk = pltpu.make_async_copy(wk_hbm, wk, sem_w.at[3])
    c_wv = pltpu.make_async_copy(wv_hbm, wv, sem_w.at[4])
    c_wo = pltpu.make_async_copy(wo_hbm, wo.at[pl.ds(0, D)], sem_w.at[5])
    c_wg = pltpu.make_async_copy(wg_hbm, wg, sem_f.at[0])
    c_wu = pltpu.make_async_copy(wu_hbm, wu, sem_f.at[1])
    c_wd = pltpu.make_async_copy(wd_hbm, wd, sem_f.at[2])

    c_wr.start()
    c_beta.start()
    x_copy(0).start()
    c_wq.start()
    c_wk.start()
    c_wv.start()
    for s in range(1, NSEG):
        x_copy(s).start()
    c_wg.start()
    c_wu.start()
    c_wd.start()
    c_wo.start()

    mask[...] = jnp.where(_iota((T, T), 0) <= _iota((T, T), 1), 0.0, NEG)
    ot[0, 0:D, :] = jnp.zeros((D, L), F32)
    c_wr.wait()
    c_beta.wait()
    wrb[...] = jnp.broadcast_to(wr[...].astype(F32).reshape(1, D), (T, D)).T
    g_row = jax.nn.sigmoid(beta[...].astype(F32).reshape(1, H))
    gate[...] = jnp.broadcast_to(g_row, (T, H)).T

    def layernorm(s):
        for c in range(NT):
            cols = slice(c * T, (c + 1) * T)
            x = xs[s, :, cols].astype(F32)
            mean = jnp.sum(x, axis=0, keepdims=True) / D
            cen = x - mean
            var = jnp.sum(cen * cen, axis=0, keepdims=True) / D
            inv = 1.0 / _round(jnp.sqrt(_round(_round(var) + EPS)))
            y = (_round(x - _round(mean)) * inv).astype(BF16)
            xn[s * NT + c] = y
            r = jnp.sum(y.astype(F32) * wrb[...], axis=0, keepdims=True)
            rr[s, :, cols] = jnp.broadcast_to(r, (8, T))

    def xn_seg(s):
        return jnp.concatenate([xn[s * NT + c] for c in range(NT)], axis=1)

    x_copy(0).wait()
    layernorm(0)
    c_wq.wait()
    c_wk.wait()
    c_wv.wait()

    def project(s, carry):
        @pl.when(s + 1 < NSEG)
        def _():
            x_copy(s + 1).wait()

        rhs = xn_seg(s)
        for lo, hi in CHUNKS:
            kt[lo:hi, :] = _dot(wk[:, lo:hi], rhs, 0, 0).astype(BF16)
        for g in range(NG):
            kg[s, g] = pltpu.bitcast(kt[_win(g):_win(g) + GW, :].T, U32)
        for lo, hi in CHUNKS:
            q = _dot(wq[:, lo:hi], rhs, 0, 0)
            qt[s, lo // 2:hi // 2, :] = pltpu.bitcast((q * QSCALE).astype(BF16), U32)
            pq[s, lo:hi, :] = _phi(q).astype(BF16)
        for lo, hi in CHUNKS:
            vt[s, lo:hi, :] = _round(_dot(wv[:, lo:hi], rhs, 0, 0))
        layernorm(jnp.minimum(s + 1, NSEG - 1))
        return carry

    lax.fori_loop(0, NSEG, project, 0)

    r = _round(rr[...])
    pos = (_iota(r.shape, 0) * L + _iota(r.shape, 2)).astype(F32)

    def top(vals, allowed):
        best = jnp.max(vals)
        idx = jnp.min(jnp.where((vals == best) & allowed, pos, float(S - 1)))
        return best, idx

    r0, p0 = top(r, pos >= 0.0)
    r1, p1 = top(jnp.where(pos == p0, -jnp.inf, r), pos != p0)
    i0 = jnp.clip(p0.astype(jnp.int32), 0, S - 1)
    i1 = jnp.clip(p1.astype(jnp.int32), 0, S - 1)

    def onehot(row, lane, shape):
        return jnp.where((_iota(shape, 0) == row) & (_iota(shape, 1) == lane), 1.0, 0.0)

    x_sel = (_dot(onehot(0, i0 % T, (16, T)).astype(BF16), xn[i0 // T], 1, 1)
             + _dot(onehot(1, i1 % T, (16, T)).astype(BF16), xn[i1 // T], 1, 1))
    for s in range(NSEG):
        ot[s, D:DE, :] = onehot(0, i0 - s * L, (16, L)) + onehot(1, i1 - s * L, (16, L))

    def head_of(d):
        return ((d >= 0).astype(jnp.int32) + (d >= DH).astype(jnp.int32)
                + (d >= 2 * DH).astype(jnp.int32) + (d >= 3 * DH).astype(jnp.int32)
                + (d >= 4 * DH).astype(jnp.int32) - 1)

    def spread(rows):
        sub = _iota((8, rows[0].shape[1]), 0)
        out = []
        for v in range(9):
            a, b = 8 * v // DH, (8 * v + 7) // DH
            full = jnp.broadcast_to(rows[a], sub.shape)
            out.append(full if a == b else jnp.where(sub < DH * b - 8 * v, full, rows[b]))
        return jnp.concatenate(out, axis=0)

    mem, nrm = {}, {}
    for s in range(NSEG - 1):
        for g in range(NG):
            pk = _phi(pltpu.bitcast(kg[s, g], BF16).astype(F32))
            upd = _dot(vt[s, 72 * g:72 * g + 72, :], pk.astype(BF16))
            z = jnp.sum(pk, axis=0, keepdims=True)
            mem[g] = upd if s == 0 else mem[g] + upd
            nrm[g] = z if s == 0 else nrm[g] + z
        for g in range(NG):
            off = 72 * g - _win(g)
            same = head_of(_iota((72, GW), 0)) == head_of(_iota((72, GW), 1) - off)
            pick = _iota((8, GW), 0) == head_of(_iota((8, GW), 1) - off)
            lhs = jnp.concatenate(
                [jnp.where(same, mem[g], 0.0), jnp.where(pick, nrm[g], 0.0)], axis=0)
            a = _dot(lhs, pq[s + 1, _win(g):_win(g) + GW, :])
            scale = []
            for i in range(4):
                gh = jnp.concatenate([gate[4 * g + i:4 * g + i + 1, :]] * NT, axis=1)
                scale.append(gh / (a[72 + i:73 + i, :] + 1e-6))
            ot[s + 1, 72 * g:72 * g + 72, :] = a[0:72, :] * spread(scale)

    c_wg.wait()
    c_wu.wait()
    c_wd.wait()
    c_wo.wait()
    xb = x_sel.astype(BF16)
    gt = _dot(xb, wg[...])
    hid = gt * jax.nn.sigmoid(gt) * _dot(xb, wu[...])
    y = _dot(hid.astype(BF16), wd[...], 1, 1)
    r_sel = jnp.where(_iota((16, D), 0) == 0, r0, r1)
    wo[D:DE, :] = (y * jax.nn.sigmoid(r_sel)).astype(BF16)

    def attention(s, carry):
        def q_weights(h, j):
            lo, w0 = DH * h, _win(h // 4)
            parts = []
            for b in range(w0, w0 + GW, 16):
                if b + 16 <= lo or b >= lo + DH:
                    parts.append(jnp.zeros((16, T), BF16))
                    continue
                u = qt[s, b // 2:b // 2 + 8, j * T:(j + 1) * T]
                row = _iota((8, T), 0) * 2 + b
                if not (lo <= b and b + 16 <= lo + DH):
                    u = jnp.where((row >= lo) & (row < lo + DH), u, jnp.zeros_like(u))
                parts.append(pltpu.bitcast(u, BF16))
            return jnp.concatenate(parts, axis=0)

        steps = [(g, j, c) for g in range(NG) for j in reversed(range(NT)) for c in range(j + 1)]
        mx, prob, acc = {}, {}, {}

        def scores(g, j, c):
            keys = pltpu.bitcast(kg[s, g, c * (T // 2):(c + 1) * (T // 2), :], BF16)
            for h in range(4 * g, 4 * g + 4):
                sc = _dot(keys, q_weights(h, j))
                if c == j:
                    sc = sc + mask[...]
                m = jnp.max(sc, axis=0, keepdims=True)
                if c > 0:
                    m = jnp.maximum(m, mx[h, j, c - 1])
                mx[h, j, c] = m
                prob[h, j, c] = jnp.exp2(sc - m).astype(BF16)

        def values(g, j, c):
            done = []
            for h in range(4 * g, 4 * g + 4):
                v0 = (DH * h // 8) * 8
                ones = 0 if DH * h > v0 else 23
                v = vt[s, v0:v0 + 24, c * T:(c + 1) * T]
                v = jnp.where(_iota((24, T), 0) == ones, 1.0, v)
                o = _dot(v, prob.pop((h, j, c)))
                if c > 0:
                    o = acc[h, j] * jnp.exp2(mx[h, j, c - 1] - mx[h, j, c]) + o
                acc[h, j] = o
                if c == j:
                    done.append(o * ((1.0 - gate[h:h + 1, :]) / o[ones:ones + 1, :]))
            if c == j:
                sub = _iota((8, T), 0)
                rows = [done[0][0:16]]
                for i in range(1, 4):
                    rows.append(jnp.where(sub < 2 * i, done[i - 1][16:24], done[i][0:8]))
                    rows.append(done[i][8:16])
                rows.append(done[3][16:24])
                ot[s, 72 * g:72 * g + 72, j * T:(j + 1) * T] += jnp.concatenate(rows, axis=0)

        for i in range(len(steps) + PV_DELAY):
            if i < len(steps):
                scores(*steps[i])
            if i >= PV_DELAY:
                values(*steps[i - PV_DELAY])
        return carry

    lax.fori_loop(0, NSEG, attention, 0)

    def finish(s, carry):
        rhs = ot[s].astype(BF16)
        for lo, hi in CHUNKS:
            res = xs[s, lo:hi, :].astype(F32) + jnp.concatenate(
                [xn[s * NT + c, lo:hi, :] for c in range(NT)], axis=1).astype(F32)
            outb[s, lo:hi, :] = (_dot(wo[:, lo:hi], rhs, 0, 0) + res).astype(BF16)
        out_copy(s).start()
        return carry

    lax.fori_loop(0, NSEG, finish, 0)
    for s in range(NSEG):
        out_copy(s).wait()


@jax.jit
def pallas_parallel_sum__memory_aug_infini_attn__moe_arch_mod__prompt_kernel(
    A_x: jax.Array,
    A_wq: jax.Array,
    A_wk: jax.Array,
    A_wv: jax.Array,
    A_wo: jax.Array,
    A_beta: jax.Array,
    B_x: jax.Array,
    B_w_r: jax.Array,
    B_w_gate: jax.Array,
    B_w_up: jax.Array,
    B_w_down: jax.Array,
):
    del B_x
    scratch = [
        pltpu.VMEM((NSEG, D, L), BF16),
        pltpu.VMEM((NSEG * NT, D, T), BF16),
        pltpu.VMEM((D, D), BF16),
        pltpu.VMEM((D, D), BF16),
        pltpu.VMEM((D, D), BF16),
        pltpu.VMEM((DE, D), BF16),
        pltpu.VMEM((H,), BF16),
        pltpu.VMEM((D,), BF16),
        pltpu.VMEM((D, FF), BF16),
        pltpu.VMEM((D, FF), BF16),
        pltpu.VMEM((D, FF), BF16),
        pltpu.VMEM((NSEG, D // 2, L), U32),
        pltpu.VMEM((NSEG, D, L), BF16),
        pltpu.VMEM((NSEG, D, L), F32),
        pltpu.VMEM((D, L), BF16),
        pltpu.VMEM((NSEG, NG, L // 2, GW), U32),
        pltpu.VMEM((NSEG, DE, L), F32),
        pltpu.VMEM((NSEG, 8, L), F32),
        pltpu.VMEM((D, T), F32),
        pltpu.VMEM((H, T), F32),
        pltpu.VMEM((T, T), F32),
        pltpu.VMEM((NSEG, D, L), BF16),
        pltpu.SemaphoreType.DMA((NSEG,)),
        pltpu.SemaphoreType.DMA((6,)),
        pltpu.SemaphoreType.DMA((3,)),
        pltpu.SemaphoreType.DMA((NSEG,)),
    ]
    out_t = pl.pallas_call(
        _kernel,
        out_shape=jax.ShapeDtypeStruct((D, S), BF16),
        in_specs=[pl.BlockSpec(memory_space=pl.ANY)] * 10,
        out_specs=pl.BlockSpec(memory_space=pl.ANY),
        scratch_shapes=scratch,
        compiler_params=pltpu.CompilerParams(vmem_limit_bytes=100 * 1024 * 1024),
        name="infini_mod",
    )(A_x.reshape(S, D).T, A_wq, A_wk, A_wv, A_wo, A_beta, B_w_r, B_w_gate, B_w_up, B_w_down.T)
    return out_t.T.reshape(1, S, D)
```

```python
import jax
import jax.numpy as jnp
import numpy as np
from jax import lax
import jax.experimental.pallas as pl
import jax.experimental.pallas.tpu as pltpu

F32, BF16, U32 = jnp.float32, jnp.bfloat16, jnp.uint32

S, D, H, NSEG, FF = 2048, 576, 32, 4, 4608
DH = D // H
L = S // NSEG
T = 128
NT = L // T
NG = H // 4
GW = 80
DE = D + 16
QSCALE = float(DH ** -0.5 * np.log2(np.e))
EPS = float(np.asarray(1e-5, dtype=jnp.bfloat16))
NEG = -1e30
CHUNKS = ((0, 128), (128, 256), (256, 384), (384, 512), (512, 576))
PV_DELAY = 2
LN_BLOCK = 144


def _dot(a, b, ca=1, cb=0):
    return lax.dot_general(a, b, (((ca,), (cb,)), ((), ())), preferred_element_type=F32)


def _iota(shape, dim):
    return lax.broadcasted_iota(jnp.int32, shape, dim)


def _round(x):
    return x.astype(BF16).astype(F32)


def _phi(t):
    return jnp.where(t > 0, t + 1.0, jnp.exp(t))


def _win(g):
    return (72 * g // 16) * 16


def _after(value, token):
    if token is None:
        return value
    return jnp.where(token * token < 0.0, 0.0, value)


def _kernel(x_hbm, wq_hbm, wk_hbm, wv_hbm, wo_hbm, beta_hbm, wr_hbm, wg_hbm, wu_hbm, wd_hbm,
            out_hbm,
            xs, xn, wq, wk, wv, wo, beta, wr, wg, wu, wd,
            qt, pq, pk, vt, kt, kg, ot, rr, wrb, gate, mask, outb,
            sem_x, sem_w, sem_o):
    def x_copy(s):
        return pltpu.make_async_copy(x_hbm.at[:, pl.ds(s * L, L)], xs.at[s], sem_x.at[s])

    out_copies = []

    def send(s, lo, hi):
        c = pltpu.make_async_copy(outb.at[s, pl.ds(lo, hi - lo)],
                                  out_hbm.at[pl.ds(lo, hi - lo), pl.ds(s * L, L)],
                                  sem_o.at[len(out_copies)])
        c.start()
        out_copies.append(c)

    c_wr = pltpu.make_async_copy(wr_hbm, wr, sem_w.at[0])
    c_beta = pltpu.make_async_copy(beta_hbm, beta, sem_w.at[1])
    c_wq = pltpu.make_async_copy(wq_hbm, wq, sem_w.at[2])
    c_wk = pltpu.make_async_copy(wk_hbm, wk, sem_w.at[3])
    c_wv = pltpu.make_async_copy(wv_hbm, wv, sem_w.at[4])
    late = [pltpu.make_async_copy(wg_hbm, wg, sem_w.at[5]),
            pltpu.make_async_copy(wu_hbm, wu, sem_w.at[6]),
            pltpu.make_async_copy(wd_hbm, wd, sem_w.at[7]),
            pltpu.make_async_copy(wo_hbm, wo.at[pl.ds(0, D)], sem_w.at[8])]

    x_copy(0).start()
    c_wr.start()
    c_beta.start()
    c_wk.start()

    mask[...] = jnp.where(_iota((T, T), 0) <= _iota((T, T), 1), 0.0, NEG)
    c_wr.wait()
    c_beta.wait()
    wrb[...] = jnp.broadcast_to(wr[...].astype(F32).reshape(1, D), (T, D)).T
    g_row = jax.nn.sigmoid(beta[...].astype(F32).reshape(1, H))
    gate[...] = jnp.broadcast_to(g_row, (T, H)).T

    def layernorm(s):
        for c in range(NT):
            cols = slice(c * T, (c + 1) * T)
            mean = jnp.sum(xs[s, :, cols].astype(F32), axis=0, keepdims=True) / D
            sq = None
            for lo in range(0, D, 2 * LN_BLOCK):
                tok = yield
                cen = xs[s, lo:lo + 2 * LN_BLOCK, cols].astype(F32) - _after(mean, tok)
                part = jnp.sum((cen * cen).reshape(-1, 8, T), axis=0)
                sq = part if sq is None else sq + part
            var = jnp.sum(sq, axis=0, keepdims=True) / D
            inv = 1.0 / _round(jnp.sqrt(_round(_round(var) + EPS)))
            r = None
            for lo in range(0, D, LN_BLOCK):
                tok = yield
                rows = slice(lo, lo + LN_BLOCK)
                y = _round(xs[s, rows, cols].astype(F32) - _after(_round(mean), tok)) * inv
                y = y.astype(BF16)
                xn[s * NT + c, rows, :] = y
                part = jnp.sum((y.astype(F32) * wrb[rows, :]).reshape(-1, 8, T), axis=0)
                r = part if r is None else r + part
            rr[s, :, cols] = jnp.broadcast_to(jnp.sum(r, axis=0, keepdims=True), (8, T))

    background = []

    def start_background(gen):
        next(gen)
        background.append(gen)

    def pace(token):
        while background:
            try:
                background[0].send(token)
                return
            except StopIteration:
                background.pop(0)
                return

    def drain():
        while background:
            pace(None)

    def project(w, s, lo, hi):
        rhs = jnp.concatenate([xn[s * NT + c] for c in range(NT)], axis=1)
        out = _dot(w[:, lo:hi], rhs, 0, 0)
        for c in range(NT):
            pace(out[-1:, c * T:(c + 1) * T])
        return out

    def head_of(d):
        h = jnp.full(d.shape, -1, jnp.int32)
        for i in range(5):
            h = jnp.where(d >= i * DH, i, h)
        return h

    own = []
    for off in (0, 8):
        row = _iota((GW, GW), 0)
        own.append(jnp.where(row < 72, head_of(row), row - 72) == head_of(_iota((GW, GW), 1) - off))
        own[-1] = own[-1] & (row < 76)

    def spread(rows):
        sub = _iota(rows.shape, 0)
        full = [jnp.broadcast_to(rows[i:i + 1], rows.shape) for i in range(4)]
        out = []
        for v in range(9):
            a, b = 8 * v // DH, (8 * v + 7) // DH
            out.append(full[a] if a == b else jnp.where(sub < DH * b - 8 * v, full[a], full[b]))
        return jnp.concatenate(out, axis=0)

    mem = {}

    def remember(s):
        for g in range(NG):
            lhs = jnp.concatenate([vt[s, 72 * g:72 * g + 72, :], jnp.ones((8, L), F32)], axis=0)
            upd = _dot(lhs, pk[s, _win(g):_win(g) + GW, :], 1, 1)
            mem[g] = upd if s == 0 else mem[g] + upd

    def recall(s):
        for g in range(NG):
            a = _dot(jnp.where(own[g % 2], mem[g], 0.0), pq[s, _win(g):_win(g) + GW, :])
            g4 = gate[8 * (g // 2):8 * (g // 2) + 8, :]
            if g % 2:
                g4 = pltpu.roll(g4, 4, 0)
            scale = jnp.concatenate([g4] * NT, axis=1) / (a[72:GW, :] + 1e-6)
            ot[s, 72 * g:72 * g + 72, :] = a[0:72, :] * spread(scale)

    def keys(s):
        for lo, hi in CHUNKS:
            k = project(wk, s, lo, hi)
            kt[s, lo:hi, :] = k.astype(BF16)
            if s + 1 < NSEG:
                pk[s, lo:hi, :] = _phi(k).astype(BF16)
        for g in range(NG):
            kg[s, g] = pltpu.bitcast(kt[s, _win(g):_win(g) + GW, :].T, U32)

    def queries(s):
        for lo, hi in CHUNKS:
            q = project(wq, s, lo, hi)
            qt[s, lo // 2:hi // 2, :] = pltpu.bitcast((q * QSCALE).astype(BF16), U32)
            if s > 0:
                pq[s, lo:hi, :] = _phi(q).astype(BF16)

    def vals(s):
        for lo, hi in CHUNKS:
            vt[s, lo:hi, :] = _round(project(wv, s, lo, hi))

    x_copy(0).wait()
    c_wq.start()
    c_wv.start()
    start_background(layernorm(0))
    drain()
    c_wk.wait()
    for s in range(1, NSEG):
        x_copy(s).start()
    keys(0)
    c_wq.wait()
    c_wv.wait()
    queries(0)
    for c in late:
        c.start()
    for s in range(1, NSEG):
        x_copy(s).wait()
    start_background(layernorm(1))
    vals(0)
    drain()
    for s in range(1, NSEG):
        if s + 1 < NSEG:
            start_background(layernorm(s + 1))
        keys(s)
        remember(s - 1)
        queries(s)
        vals(s)
        drain()
        recall(s)

    r = _round(rr[...])
    pos = (_iota(r.shape, 0) * L + _iota(r.shape, 2)).astype(F32)

    def top(vals, allowed):
        best = jnp.max(vals)
        idx = jnp.min(jnp.where((vals == best) & allowed, pos, float(S - 1)))
        return best, idx

    r0, p0 = top(r, pos >= 0.0)
    r1, p1 = top(jnp.where(pos == p0, -jnp.inf, r), pos != p0)
    i0 = jnp.clip(p0.astype(jnp.int32), 0, S - 1)
    i1 = jnp.clip(p1.astype(jnp.int32), 0, S - 1)

    def onehot(row, lane, shape):
        return jnp.where((_iota(shape, 0) == row) & (_iota(shape, 1) == lane), 1.0, 0.0)

    x_sel = (_dot(onehot(0, i0 % T, (8, T)), xn[i0 // T], 1, 1)
             + _dot(onehot(1, i1 % T, (8, T)), xn[i1 // T], 1, 1))
    for s in range(NSEG):
        ot[s, D:DE, :] = onehot(0, i0 - s * L, (16, L)) + onehot(1, i1 - s * L, (16, L))

    def ffn():
        hid, y = {}, {}

        def up(i):
            acc = []
            for w in (wg, wu):
                part = None
                for lo, hi in CHUNKS:
                    t = _dot(x_sel[:, lo:hi], w[lo:hi, i * T:(i + 1) * T])
                    part = t if part is None else part + t
                    yield
                acc.append(part)
            hid[i] = _round(acc[0] * jax.nn.sigmoid(acc[0]) * acc[1])

        def down(i):
            for lo, hi in CHUNKS:
                t = _dot(hid[i], wd[lo:hi, i * T:(i + 1) * T], 1, 1)
                y[lo] = t if i == 0 else y[lo] + t
                yield

        n = FF // T
        for i in range(n + 2):
            if i < n:
                yield from up(i)
            if i >= 2:
                yield from down(i - 2)
        out = jnp.concatenate([y[lo] for lo, _ in CHUNKS], axis=1)
        r_sel = jnp.where(_iota((8, D), 0) == 0, r0, r1)
        out = out * jax.nn.sigmoid(r_sel)
        wo[D:DE, :] = jnp.concatenate([out, jnp.zeros((8, D), F32)], axis=0).astype(BF16)

    def q_weights(s, h, j):
        lo, w0 = DH * h, _win(h // 4)
        parts = []
        for b in range(w0, w0 + GW, 16):
            if b + 16 <= lo or b >= lo + DH:
                parts.append(jnp.zeros((16, T), BF16))
                continue
            u = qt[s, b // 2:b // 2 + 8, j * T:(j + 1) * T]
            row = _iota((8, T), 0) * 2 + b
            if not (lo <= b and b + 16 <= lo + DH):
                u = jnp.where((row >= lo) & (row < lo + DH), u, jnp.zeros_like(u))
            parts.append(pltpu.bitcast(u, BF16))
        return jnp.concatenate(parts, axis=0)

    mx, prob, acc = {}, {}, {}

    def scores(s, g, j, c):
        k = pltpu.bitcast(kg[s, g, c * (T // 2):(c + 1) * (T // 2), :], BF16)
        for h in range(4 * g, 4 * g + 4):
            sc = _dot(k, q_weights(s, h, j))
            if c == j:
                sc = sc + mask[...]
            m = jnp.max(sc, axis=0, keepdims=True)
            if c > 0:
                m = jnp.maximum(m, mx[s, h, j, c - 1])
            mx[s, h, j, c] = m
            prob[s, h, j, c] = jnp.exp2(sc - m).astype(BF16)

    def values(s, g, j, c):
        done = []
        for h in range(4 * g, 4 * g + 4):
            v0 = (DH * h // 8) * 8
            ones = 0 if DH * h > v0 else 23
            v = vt[s, v0:v0 + 24, c * T:(c + 1) * T]
            v = jnp.where(_iota((24, T), 0) == ones, 1.0, v)
            o = _dot(v, prob.pop((s, h, j, c)))
            if c > 0:
                o = acc[h] * jnp.exp2(mx[s, h, j, c - 1] - mx[s, h, j, c]) + o
            acc[h] = o
            if c == j:
                done.append(o * ((1.0 - gate[h:h + 1, :]) / o[ones:ones + 1, :]))
        if c == j:
            sub = _iota((8, T), 0)
            rows = [done[0][0:16]]
            for i in range(1, 4):
                rows.append(jnp.where(sub < 2 * i, done[i - 1][16:24], done[i][0:8]))
                rows.append(done[i][8:16])
            rows.append(done[3][16:24])
            o = jnp.concatenate(rows, axis=0)
            at = (s, slice(72 * g, 72 * g + 72), slice(j * T, (j + 1) * T))
            ot[at] = o if s == 0 else ot[at] + o

    def attention(segs, extra=None):
        steps = [(s, g, j, c) for s in segs for g in range(NG)
                 for j in reversed(range(NT)) for c in range(j + 1)]
        for i in range(len(steps) + PV_DELAY):
            if i < len(steps):
                scores(*steps[i])
            if i >= PV_DELAY:
                values(*steps[i - PV_DELAY])
            if extra is not None:
                for _ in range(4):
                    next(extra, None)

    def finish(s):
        rhs = ot[s].astype(BF16)
        for lo, hi in CHUNKS:
            res = xs[s, lo:hi, :].astype(F32) + jnp.concatenate(
                [xn[s * NT + c, lo:hi, :] for c in range(NT)], axis=1).astype(F32)
            outb[s, lo:hi, :] = (_dot(wo[:, lo:hi], rhs, 0, 0) + res).astype(BF16)
            if s == NSEG - 1 and hi >= 4 * T:
                send(s, 0 if hi < D else lo, hi)
        if s < NSEG - 1:
            send(s, 0, D)

    attention([0])
    for c in late:
        c.wait()
    routed = ffn()
    attention([1, 2, 3], routed)
    for _ in routed:
        pass
    for s in range(NSEG):
        finish(s)
    for c in out_copies:
        c.wait()


@jax.jit
def pallas_parallel_sum__memory_aug_infini_attn__moe_arch_mod__prompt_kernel(
    A_x: jax.Array,
    A_wq: jax.Array,
    A_wk: jax.Array,
    A_wv: jax.Array,
    A_wo: jax.Array,
    A_beta: jax.Array,
    B_x: jax.Array,
    B_w_r: jax.Array,
    B_w_gate: jax.Array,
    B_w_up: jax.Array,
    B_w_down: jax.Array,
):
    del B_x
    scratch = [
        pltpu.VMEM((NSEG, D, L), BF16),
        pltpu.VMEM((NSEG * NT, D, T), BF16),
        pltpu.VMEM((D, D), BF16),
        pltpu.VMEM((D, D), BF16),
        pltpu.VMEM((D, D), BF16),
        pltpu.VMEM((DE, D), BF16),
        pltpu.VMEM((H,), BF16),
        pltpu.VMEM((D,), BF16),
        pltpu.VMEM((D, FF), BF16),
        pltpu.VMEM((D, FF), BF16),
        pltpu.VMEM((D, FF), BF16),
        pltpu.VMEM((NSEG, D // 2, L), U32),
        pltpu.VMEM((NSEG, D, L), BF16),
        pltpu.VMEM((NSEG, D, L), BF16),
        pltpu.VMEM((NSEG, D, L), F32),
        pltpu.VMEM((NSEG, D, L), BF16),
        pltpu.VMEM((NSEG, NG, L // 2, GW), U32),
        pltpu.VMEM((NSEG, DE, L), F32),
        pltpu.VMEM((NSEG, 8, L), F32),
        pltpu.VMEM((D, T), F32),
        pltpu.VMEM((H, T), F32),
        pltpu.VMEM((T, T), F32),
        pltpu.VMEM((NSEG, D, L), BF16),
        pltpu.SemaphoreType.DMA((NSEG,)),
        pltpu.SemaphoreType.DMA((9,)),
        pltpu.SemaphoreType.DMA((NSEG + 1,)),
    ]
    out_t = pl.pallas_call(
        _kernel,
        out_shape=jax.ShapeDtypeStruct((D, S), BF16),
        in_specs=[pl.BlockSpec(memory_space=pl.ANY)] * 10,
        out_specs=pl.BlockSpec(memory_space=pl.ANY),
        scratch_shapes=scratch,
        compiler_params=pltpu.CompilerParams(vmem_limit_bytes=100 * 1024 * 1024),
        name="infini_mod",
    )(A_x.reshape(S, D).T, A_wq, A_wk, A_wv, A_wo, A_beta, B_w_r, B_w_gate, B_w_up, B_w_down.T)
    return out_t.T.reshape(1, S, D)
```

```python
import jax
import jax.numpy as jnp
import numpy as np
from jax import lax
import jax.experimental.pallas as pl
import jax.experimental.pallas.tpu as pltpu

F32, BF16, U32 = jnp.float32, jnp.bfloat16, jnp.uint32

S, D, H, NSEG, FF = 2048, 576, 32, 4, 4608
DH = D // H
L = S // NSEG
T = 128
NT = L // T
NG = H // 4
GW = 80
DE = D + 16
QSCALE = float(DH ** -0.5 * np.log2(np.e))
EPS = float(np.asarray(1e-5, dtype=jnp.bfloat16))
NEG = -1e30
CHUNKS = ((0, 128), (128, 256), (256, 384), (384, 512), (512, 576))
PV_DELAY = 2
FFN_RATE = (4, 4, 0)
LN_BLOCK = 144
MC = 192


def _dot(a, b, ca=1, cb=0):
    return lax.dot_general(a, b, (((ca,), (cb,)), ((), ())), preferred_element_type=F32)


def _iota(shape, dim):
    return lax.broadcasted_iota(jnp.int32, shape, dim)


def _round(x):
    return x.astype(BF16).astype(F32)


def _phi(t):
    return jnp.where(t > 0, t + 1.0, jnp.exp(t))


def _win(g):
    return (72 * g // 16) * 16


def _after(value, token):
    if token is None:
        return value
    return jnp.where(token * token < 0.0, 0.0, value)


def _kernel(x_hbm, wq_hbm, wk_hbm, wv_hbm, wo_hbm, beta_hbm, wr_hbm, wg_hbm, wu_hbm, wd_hbm,
            out_hbm,
            xs, xn, wq, wk, wv, wo, beta, wr, wg, wu, wd,
            wqt, wkt, wvt, wot, qt, pq, pk, vt, kt, kg, ot, rr, wrb, gate, mask, outb,
            sem_x, sem_w, sem_o):
    def x_copy(s):
        return pltpu.make_async_copy(x_hbm.at[:, pl.ds(s * L, L)], xs.at[s], sem_x.at[s])

    out_copies = []

    def send(s, lo, hi):
        c = pltpu.make_async_copy(outb.at[s, :, pl.ds(lo, hi - lo)],
                                  out_hbm.at[:, pl.ds(s * L + lo, hi - lo)],
                                  sem_o.at[len(out_copies)])
        c.start()
        out_copies.append(c)

    c_wr = pltpu.make_async_copy(wr_hbm, wr, sem_w.at[0])
    c_beta = pltpu.make_async_copy(beta_hbm, beta, sem_w.at[1])
    c_wq = pltpu.make_async_copy(wq_hbm, wq, sem_w.at[2])
    c_wk = pltpu.make_async_copy(wk_hbm, wk, sem_w.at[3])
    c_wv = pltpu.make_async_copy(wv_hbm, wv, sem_w.at[4])
    late = [pltpu.make_async_copy(wg_hbm, wg, sem_w.at[5]),
            pltpu.make_async_copy(wu_hbm, wu, sem_w.at[6]),
            pltpu.make_async_copy(wd_hbm, wd, sem_w.at[7]),
            pltpu.make_async_copy(wo_hbm, wo.at[pl.ds(0, D)], sem_w.at[8])]

    xr = [x_copy(s) for s in range(1, NSEG)]
    for c in [c_wr, c_beta, x_copy(0), c_wk]:
        c.start()

    key, qry = _iota((T // 2, T), 0), _iota((T // 2, T), 1)
    mask[0] = jnp.where(key <= qry, 0.0, NEG)
    mask[1] = jnp.where(key <= (qry ^ (T // 2)), 0.0, NEG)
    mask[2] = jnp.where(key <= (qry & (T // 2 - 1)), 0.0, NEG)
    c_wr.wait()
    c_beta.wait()
    wrb[...] = jnp.broadcast_to(wr[...].astype(F32).reshape(1, D), (T, D)).T
    g_row = jax.nn.sigmoid(beta[...].astype(F32).reshape(1, H))
    gate[...] = jnp.broadcast_to(g_row, (T, H)).T

    def layernorm(s):
        for c in range(NT):
            cols = slice(c * T, (c + 1) * T)
            mean = jnp.sum(xs[s, :, cols].astype(F32), axis=0, keepdims=True) / D
            sq = None
            for lo in range(0, D, 2 * LN_BLOCK):
                tok = yield
                cen = xs[s, lo:lo + 2 * LN_BLOCK, cols].astype(F32) - _after(mean, tok)
                part = jnp.sum((cen * cen).reshape(-1, 8, T), axis=0)
                sq = part if sq is None else sq + part
            var = jnp.sum(sq, axis=0, keepdims=True) / D
            inv = 1.0 / _round(jnp.sqrt(_round(_round(var) + EPS)))
            r = None
            for lo in range(0, D, LN_BLOCK):
                tok = yield
                rows = slice(lo, lo + LN_BLOCK)
                y = _round(xs[s, rows, cols].astype(F32) - _after(_round(mean), tok)) * inv
                y = y.astype(BF16)
                xn[s * NT + c, rows, :] = y
                part = jnp.sum((y.astype(F32) * wrb[rows, :]).reshape(-1, 8, T), axis=0)
                r = part if r is None else r + part
            rr[s, :, cols] = jnp.broadcast_to(jnp.sum(r, axis=0, keepdims=True), (8, T))

    background = []

    def start_background(gen):
        next(gen)
        background.append(gen)

    def pace(token):
        while background:
            try:
                background[0].send(token)
                return
            except StopIteration:
                background.pop(0)
                return

    def drain():
        while background:
            pace(None)

    def transpose_weights(src, dst):
        for lo, hi in CHUNKS:
            dst[lo // 2:hi // 2, :] = pltpu.bitcast(src[:, lo:hi].T, U32)

    deferred = []

    later = []

    def flush():
        while deferred:
            deferred.pop(0)()
        if later:
            later.pop(0)()

    def project(wt, rhs_of, consume, paced=False, sync=None, sync_at=D - MC):
        for c in range(NT):
            rhs = rhs_of(c)
            for lo in range(0, D, MC):
                out = _dot(pltpu.bitcast(wt[lo // 2:(lo + MC) // 2, :], BF16), rhs)
                if sync is not None and (c, lo) == (NT - 1, sync_at):
                    sync()
                flush()

                def post(c=c, lo=lo, out=out):
                    consume(slice(c * T, (c + 1) * T), lo, out)
                    if paced:
                        pace(out[-1:])

                deferred.append(post)

    def head_of(d):
        h = jnp.full(d.shape, -1, jnp.int32)
        for i in range(5):
            h = jnp.where(d >= i * DH, i, h)
        return h

    own = []
    for off in (0, 8):
        row = _iota((GW, GW), 0)
        own.append(jnp.where(row < 72, head_of(row), row - 72) == head_of(_iota((GW, GW), 1) - off))
        own[-1] = own[-1] & (row < 76)

    def spread(rows):
        sub = _iota(rows.shape, 0)
        full = [jnp.broadcast_to(rows[i:i + 1], rows.shape) for i in range(4)]
        out = []
        for v in range(9):
            a, b = 8 * v // DH, (8 * v + 7) // DH
            out.append(full[a] if a == b else jnp.where(sub < DH * b - 8 * v, full[a], full[b]))
        return jnp.concatenate(out, axis=0)

    mem = {}

    def remember(s):
        for g in range(NG):
            lhs = jnp.concatenate([vt[s, 72 * g:72 * g + 72, :], jnp.ones((8, L), F32)], axis=0)
            upd = _dot(lhs, pk[s, _win(g):_win(g) + GW, :], 1, 1)
            mem[g] = upd if s == 0 else mem[g] + upd
            flush()

    def recall(s):
        for g in range(NG):
            lhs = jnp.where(own[g % 2], mem[g], 0.0)
            g4 = gate[8 * (g // 2):8 * (g // 2) + 8, :]
            if g % 2:
                g4 = pltpu.roll(g4, 4, 0)
            for c in range(NT):
                cols = slice(c * T, (c + 1) * T)
                a = _dot(lhs, pq[s, _win(g):_win(g) + GW, cols])
                ot[s, 72 * g:72 * g + 72, cols] = a[0:72, :] * spread(g4 / (a[72:GW, :] + 1e-6))
            flush()

    def keys(s, **kw):
        def consume(cols, lo, k):
            kt[s, lo:lo + MC, cols] = k.astype(BF16)
            if s + 1 < NSEG:
                pk[s, lo:lo + MC, cols] = _phi(k).astype(BF16)
            if lo + MC == D:
                for g in range(NG):
                    kg[s, g, cols.start // 2:cols.stop // 2, :] = pltpu.bitcast(
                        kt[s, _win(g):_win(g) + GW, cols].T, U32)

        project(wkt, lambda c: xn[s * NT + c], consume, **kw)

    def queries(s, **kw):
        def consume(cols, lo, q):
            qt[s, lo // 2:(lo + MC) // 2, cols] = pltpu.bitcast((q * QSCALE).astype(BF16), U32)
            if s > 0:
                pq[s, lo:lo + MC, cols] = _phi(q).astype(BF16)

        project(wqt, lambda c: xn[s * NT + c], consume, **kw)

    def vals(s, **kw):
        def consume(cols, lo, v):
            vt[s, lo:lo + MC, cols] = _round(v)

        project(wvt, lambda c: xn[s * NT + c], consume, **kw)

    picked = []

    def onehot(row, lane, shape):
        return jnp.where((_iota(shape, 0) == row) & (_iota(shape, 1) == lane), 1.0, 0.0)

    def route():
        tok = yield
        r = _after(_round(rr[...]), tok[:, 0:1])
        pos = (_iota(r.shape, 0) * L + _iota(r.shape, 2)).astype(F32)

        def top(vals, allowed):
            best = jnp.max(vals)
            return best, jnp.min(jnp.where((vals == best) & allowed, pos, float(S - 1)))

        r0, p0 = top(r, pos >= 0.0)
        r1, p1 = top(jnp.where(pos == p0, -jnp.inf, r), pos != p0)
        i0 = jnp.clip(p0.astype(jnp.int32), 0, S - 1)
        i1 = jnp.clip(p1.astype(jnp.int32), 0, S - 1)
        picked.extend([(r0, i0), (r1, i1)])
        for s in range(NSEG):
            ot[s, D:DE, :] = onehot(0, i0 - s * L, (16, L)) + onehot(1, i1 - s * L, (16, L))

    def ffn():
        (r0, i0), (r1, i1) = picked
        x_sel = (_dot(onehot(0, i0 % T, (8, T)), xn[i0 // T], 1, 1)
                 + _dot(onehot(1, i1 % T, (8, T)), xn[i1 // T], 1, 1))
        for _ in range(12):
            yield
        hid, y = {}, {}

        def up(i):
            acc = []
            for w in (wg, wu):
                part = None
                for lo, hi in CHUNKS:
                    t = _dot(x_sel[:, lo:hi], w[lo:hi, i * T:(i + 1) * T])
                    part = t if part is None else part + t
                    yield
                acc.append(part)
            hid[i] = _round(acc[0] * jax.nn.sigmoid(acc[0]) * acc[1])

        def down(i):
            for lo, hi in CHUNKS:
                t = _dot(hid[i], wd[lo:hi, i * T:(i + 1) * T], 1, 1)
                y[lo] = t if i == 0 else y[lo] + t
                yield

        n = FF // T
        for i in range(n + 2):
            if i < n:
                yield from up(i)
            if i >= 2:
                yield from down(i - 2)
        out = jnp.concatenate([y[lo] for lo, _ in CHUNKS], axis=1)
        r_sel = jnp.where(_iota((8, D), 0) == 0, r0, r1)
        out = out * jax.nn.sigmoid(r_sel)
        wo[D:DE, :] = jnp.concatenate([out, jnp.zeros((8, D), F32)], axis=0).astype(BF16)
        transpose_weights(wo, wot)

    def q_rows(s, h, j):
        lo, w0 = DH * h, _win(h // 4)
        parts = []
        for b in range(w0, w0 + GW, 16):
            if b + 16 <= lo or b >= lo + DH:
                parts.append(None)
                continue
            u = qt[s, b // 2:b // 2 + 8, j * T:(j + 1) * T]
            row = _iota((8, T), 0) * 2 + b
            if not (lo <= b and b + 16 <= lo + DH):
                u = jnp.where((row >= lo) & (row < lo + DH), u, jnp.zeros_like(u))
            parts.append(pltpu.roll(u, T // 2, 1) if h % 2 else u)
        return parts

    def weights(parts):
        return jnp.concatenate([jnp.zeros((16, T), BF16) if p is None else pltpu.bitcast(p, BF16)
                                for p in parts], axis=0)

    def upper(a, b):
        ref = b if a is None else a
        a, b = (jnp.zeros_like(ref) if t is None else t for t in (a, b))
        return jnp.where(_iota(ref.shape, 1) >= T // 2, a, b)

    mx, prob, acc = {}, {}, {}

    def running_max(s, h, j, c, m):
        mx[s, h, j, c] = m if c == 0 else jnp.maximum(m, mx[s, h, j, c - 1])
        return mx[s, h, j, c]

    def scores(s, g, j, c):
        def k_rows(lo, n):
            return pltpu.bitcast(kg[s, g, lo // 2:(lo + n) // 2, :], BF16)

        if c < j:
            for h in range(4 * g, 4 * g + 4):
                sc = _dot(k_rows(c * T, T), weights(q_rows(s, h, j)))
                m = running_max(s, h, j, c, jnp.max(sc, axis=0, keepdims=True))
                prob[s, h, j, c] = jnp.exp2(sc - m).astype(BF16)
            return
        for a in range(4 * g, 4 * g + 4, 2):
            b = a + 1
            qa, qb = q_rows(s, a, j), q_rows(s, b, j)
            both = [None if p is None and t is None else upper(p, t) for p, t in zip(qa, qb)]
            sa = _dot(k_rows(c * T, T // 2), weights(qa)) + mask[0]
            sb = _dot(k_rows(c * T, T // 2), weights(qb)) + mask[1]
            sc = _dot(k_rows(c * T + T // 2, T // 2), weights(both)) + mask[2]
            mc = jnp.max(sc, axis=0, keepdims=True)
            low = jnp.full_like(mc, NEG)
            ma = jnp.maximum(jnp.max(sa, axis=0, keepdims=True), upper(mc, low))
            mb = jnp.maximum(jnp.max(sb, axis=0, keepdims=True), upper(low, mc))
            ma, mb = running_max(s, a, j, c, ma), running_max(s, b, j, c, mb)
            pc = jnp.exp2(sc - upper(ma, mb))
            prob[s, a, j, c] = jnp.concatenate(
                [jnp.exp2(sa - ma), upper(pc, None)], axis=0).astype(BF16)
            prob[s, b, j, c] = jnp.concatenate(
                [jnp.exp2(sb - mb), upper(None, pc)], axis=0).astype(BF16)

    def values(s, g, j, c):
        done = []
        for h in range(4 * g, 4 * g + 4):
            v0 = (DH * h // 8) * 8
            ones = 0 if DH * h > v0 else 23
            v = vt[s, v0:v0 + 24, c * T:(c + 1) * T]
            v = jnp.where(_iota((24, T), 0) == ones, 1.0, v)
            o = _dot(v, prob.pop((s, h, j, c)))
            if c > 0:
                o = acc[h] * jnp.exp2(mx[s, h, j, c - 1] - mx[s, h, j, c]) + o
            acc[h] = o
            if c == j:
                o = o * ((1.0 - gate[h:h + 1, :]) / o[ones:ones + 1, :])
                done.append(pltpu.roll(o, T // 2, 1) if h % 2 else o)
        if c == j:
            sub = _iota((8, T), 0)
            rows = [done[0][0:16]]
            for i in range(1, 4):
                rows.append(jnp.where(sub < 2 * i, done[i - 1][16:24], done[i][0:8]))
                rows.append(done[i][8:16])
            rows.append(done[3][16:24])
            o = jnp.concatenate(rows, axis=0)
            at = (s, slice(72 * g, 72 * g + 72), slice(j * T, (j + 1) * T))
            ot[at] = o if s == 0 else ot[at] + o

    def attention(segs, hook):
        steps = [(s, g, j, c) for s in segs for g in range(NG)
                 for j in reversed(range(NT)) for c in range(j + 1)]
        for i in range(len(steps)):
            scores(*steps[i])
            flush()
            if i >= PV_DELAY:
                s, g, j, c = steps[i - PV_DELAY]
                values(s, g, j, c)
                hook(i - PV_DELAY, mx[s, 4 * g, j, c])
        late_steps = steps[-PV_DELAY:]

        def tail():
            values(*late_steps.pop(0))
            if late_steps:
                later.append(tail)

        later.append(tail)

    def finish(s):
        def consume(cols, lo, o):
            rows = slice(lo, lo + MC)
            res = xs[s, rows, cols].astype(F32) + xn[s * NT + cols.start // T, rows, :].astype(F32)
            outb[s, rows, cols] = (o + res).astype(BF16)
            if lo + MC == D:
                if s < NSEG - 1 and cols.stop == L:
                    send(s, 0, L)
                if s == NSEG - 1 and cols.stop >= L - T:
                    send(s, 0 if cols.stop < L else cols.start, cols.stop)

        project(wot, lambda c: ot[s, :, c * T:(c + 1) * T].astype(BF16), consume)

    x_copy(0).wait()
    c_wq.start()
    c_wv.start()
    start_background(layernorm(0))
    drain()
    c_wk.wait()
    transpose_weights(wk, wkt)

    def second_wave():
        c_wq.wait()
        for c in xr:
            c.start()
        c_wv.wait()
        transpose_weights(wq, wqt)
        transpose_weights(wv, wvt)

    def third_wave():
        xr[0].wait()
        xr[1].wait()
        for c in late:
            c.start()
        xr[2].wait()

    def last_wave():
        for c in late:
            c.wait()

    keys(0, sync=second_wave, sync_at=MC)
    queries(0)
    vals(0, sync=third_wave)
    start_background(layernorm(1))
    attention([0], lambda i, token: pace(token) if i % 3 == 0 else None)
    drain()
    for s in range(1, NSEG):
        keys(s)
        remember(s - 1)
        start_background(layernorm(s + 1) if s + 1 < NSEG else route())
        vals(s, paced=True)
        queries(s, paced=True, sync=last_wave if s + 1 == NSEG else None)
        flush()
        drain()
        recall(s)

    routed = ffn()

    def ffn_steps(i, token):
        for _ in range(FFN_RATE[i % len(FFN_RATE)]):
            next(routed, None)

    attention([1, 2, 3], ffn_steps)
    for _ in routed:
        pass
    for s in range(NSEG):
        finish(s)
    flush()
    for c in out_copies:
        c.wait()


@jax.jit
def pallas_parallel_sum__memory_aug_infini_attn__moe_arch_mod__prompt_kernel(
    A_x: jax.Array,
    A_wq: jax.Array,
    A_wk: jax.Array,
    A_wv: jax.Array,
    A_wo: jax.Array,
    A_beta: jax.Array,
    B_x: jax.Array,
    B_w_r: jax.Array,
    B_w_gate: jax.Array,
    B_w_up: jax.Array,
    B_w_down: jax.Array,
):
    del B_x
    scratch = [
        pltpu.VMEM((NSEG, D, L), BF16),
        pltpu.VMEM((NSEG * NT, D, T), BF16),
        pltpu.VMEM((D, D), BF16),
        pltpu.VMEM((D, D), BF16),
        pltpu.VMEM((D, D), BF16),
        pltpu.VMEM((DE, D), BF16),
        pltpu.VMEM((H,), BF16),
        pltpu.VMEM((D,), BF16),
        pltpu.VMEM((D, FF), BF16),
        pltpu.VMEM((D, FF), BF16),
        pltpu.VMEM((D, FF), BF16),
        pltpu.VMEM((D // 2, D), U32),
        pltpu.VMEM((D // 2, D), U32),
        pltpu.VMEM((D // 2, D), U32),
        pltpu.VMEM((D // 2, DE), U32),
        pltpu.VMEM((NSEG, D // 2, L), U32),
        pltpu.VMEM((NSEG, D, L), BF16),
        pltpu.VMEM((NSEG, D, L), BF16),
        pltpu.VMEM((NSEG, D, L), F32),
        pltpu.VMEM((NSEG, D, L), BF16),
        pltpu.VMEM((NSEG, NG, L // 2, GW), U32),
        pltpu.VMEM((NSEG, DE, L), F32),
        pltpu.VMEM((NSEG, 8, L), F32),
        pltpu.VMEM((D, T), F32),
        pltpu.VMEM((H, T), F32),
        pltpu.VMEM((3, T // 2, T), F32),
        pltpu.VMEM((NSEG, D, L), BF16),
        pltpu.SemaphoreType.DMA((NSEG,)),
        pltpu.SemaphoreType.DMA((9,)),
        pltpu.SemaphoreType.DMA((NSEG + 1,)),
    ]
    out_t = pl.pallas_call(
        _kernel,
        out_shape=jax.ShapeDtypeStruct((D, S), BF16),
        in_specs=[pl.BlockSpec(memory_space=pl.ANY)] * 10,
        out_specs=pl.BlockSpec(memory_space=pl.ANY),
        scratch_shapes=scratch,
        compiler_params=pltpu.CompilerParams(vmem_limit_bytes=100 * 1024 * 1024),
        name="infini_mod",
    )(A_x.reshape(S, D).T, A_wq, A_wk, A_wv, A_wo, A_beta, B_w_r, B_w_gate, B_w_up, B_w_down.T)
    return out_t.T.reshape(1, S, D)
```

```python
import jax
import jax.numpy as jnp
import numpy as np
from jax import lax
import jax.experimental.pallas as pl
import jax.experimental.pallas.tpu as pltpu

F32, BF16, U32 = jnp.float32, jnp.bfloat16, jnp.uint32

S, D, H, NSEG, FF = 2048, 576, 32, 4, 4608
DH = D // H
L = S // NSEG
T = 128
NT = L // T
NG = H // 4
GF = 4 * DH
GW = 80
DE = D + 16
QSCALE = float(DH ** -0.5 * np.log2(np.e))
EPS = float(np.asarray(1e-5, dtype=jnp.bfloat16))
NEG = -1e30
CHUNKS = ((0, 128), (128, 256), (256, 384), (384, 512), (512, 576))
MC = 192
BLOCKS = tuple((c, lo, lo + MC) for c in range(NT) for lo in range(0, D, MC))
LN_BLOCK = 144

TILES = ((3, 0), (0, 0), (3, 1), (3, 2), (3, 3), (1, 0), (1, 1), (2, 0), (2, 1), (2, 2))
FFN_RATE = (4, 4, 0, 4, 0, 4, 4, 0, 4, 0)
PV_DELAY = 2
NB = 4
B = T // NB
PASSES = (
    (0, (0, 0, 0, 0)), (0, (1, 1, 1, 1)), (0, (2, 2, 2, 2)), (0, (3, 3, 3, 3)),
    (1, (3, 0, 0, 0)), (1, (1, 3, 1, 1)), (1, (2, 2, 3, 2)),
    (2, (2, 2, 0, 0)), (2, (1, 3, 3, 1)),
    (3, (1, 2, 3, 0)),
)


def _dot(a, b, ca=1, cb=0):
    return lax.dot_general(a, b, (((ca,), (cb,)), ((), ())), preferred_element_type=F32)


def _iota(shape, dim):
    return lax.broadcasted_iota(jnp.int32, shape, dim)


def _round(x):
    return x.astype(BF16).astype(F32)


def _phi(t):
    return jnp.where(t > 0, t + 1.0, jnp.exp(t))


def _win(g):
    return (GF * g // 16) * 16


def _after(value, token):
    if token is None:
        return value
    return jnp.where(token * token < 0.0, 0.0, value)


def _by_block(vals):
    ref = next(v for v in vals if v is not None)
    groups = []
    for p, v in enumerate(vals):
        for got, ps in groups:
            if got is v:
                ps.append(p)
                break
        else:
            groups.append((v, [p]))
    groups.sort(key=lambda e: -len(e[1]))
    block = _iota(ref.shape, 1) // B
    out = None
    for v, ps in groups:
        v = jnp.zeros_like(ref) if v is None else v
        bits = sum(1 << p for p in ps)
        out = v if out is None else jnp.where(((bits >> block) & 1) == 1, v, out)
    return out


def _onehot(row, lane, shape):
    return jnp.where((_iota(shape, 0) == row) & (_iota(shape, 1) == lane), 1.0, 0.0)


def _head_of(d):
    h = jnp.full(d.shape, -1, jnp.int32)
    for i in range(5):
        h = jnp.where(d >= i * DH, i, h)
    return h


def _spread(rows):
    sub = _iota(rows.shape, 0)
    full = [jnp.broadcast_to(rows[i:i + 1], rows.shape) for i in range(4)]
    out = []
    for v in range(GF // 8):
        a, b = 8 * v // DH, (8 * v + 7) // DH
        out.append(full[a] if a == b else jnp.where(sub < DH * b - 8 * v, full[a], full[b]))
    return jnp.concatenate(out, axis=0)


def _kernel(x_hbm, wq_hbm, wk_hbm, wv_hbm, wo_hbm, beta_hbm, wr_hbm, wg_hbm, wu_hbm, wd_hbm,
            out_hbm,
            xs, xn, wq, wk, wv, wo, beta, wr, wg, wu, wd,
            wqt, wkt, wvt, wot, qt, pq, pk, vt, kt, kg, ot, rr, wrb, gate, mask, outb,
            sem_x, sem_w, sem_o):
    def x_copy(s, lo, hi, sem):
        return pltpu.make_async_copy(x_hbm.at[:, pl.ds(s * L + lo, hi - lo)],
                                     xs.at[s, :, pl.ds(lo, hi - lo)], sem_x.at[sem])

    x_head, x_tail = x_copy(0, 0, L // 2, 0), x_copy(0, L // 2, L, 1)
    x_rest = [x_copy(s, 0, L, s + 1) for s in range(1, NSEG)]
    c_wr, c_beta, c_wq, c_wk, c_wv, *late = [
        pltpu.make_async_copy(src, dst, sem_w.at[i]) for i, (src, dst) in enumerate((
            (wr_hbm, wr), (beta_hbm, beta), (wq_hbm, wq), (wk_hbm, wk), (wv_hbm, wv),
            (wg_hbm, wg), (wu_hbm, wu), (wd_hbm, wd), (wo_hbm, wo.at[pl.ds(0, D)])))]
    out_copies = []

    def send(s, r0, r1, c0, c1):
        c = pltpu.make_async_copy(outb.at[s, pl.ds(r0, r1 - r0), pl.ds(c0, c1 - c0)],
                                  out_hbm.at[pl.ds(r0, r1 - r0), pl.ds(s * L + c0, c1 - c0)],
                                  sem_o.at[len(out_copies)])
        c.start()
        out_copies.append(c)

    def wave(wait, start=(), then=None):
        def sync():
            for c in start:
                c.start()
            for c in wait:
                c.wait()
            if then is not None:
                then()
        return sync

    for c in (c_wr, c_beta, x_head, c_wk, x_tail):
        c.start()

    key, lane = _iota((B, T), 0), _iota((B, T), 1)
    for n, (kb, heads) in enumerate(PASSES):
        shift = _by_block([jnp.full((B, T), ((p - a) % NB - p) * B) for p, a in enumerate(heads)])
        mask[n] = jnp.where(key + kb * B <= lane + shift, 0.0, NEG)
    c_wr.wait()
    c_beta.wait()
    wrb[...] = jnp.broadcast_to(wr[...].astype(F32).reshape(1, D), (T, D)).T
    g_row = jax.nn.sigmoid(beta[...].astype(F32).reshape(1, H))
    gate[...] = jnp.broadcast_to(g_row, (T, H)).T

    background = []
    deferred = []
    later = []

    def start_background(gen):
        next(gen)
        background.append(gen)

    def pace(token):
        if background:
            try:
                background[0].send(token)
            except StopIteration:
                background.pop(0)

    def drain():
        while background:
            pace(None)

    def flush():
        while deferred:
            deferred.pop(0)()
        if later:
            later.pop(0)()

    def layernorm(s, tiles=range(NT)):
        for c in tiles:
            cols = slice(c * T, (c + 1) * T)
            mean = jnp.sum(xs[s, :, cols].astype(F32), axis=0, keepdims=True) / D
            sq = None
            for lo in range(0, D, 2 * LN_BLOCK):
                tok = yield
                cen = xs[s, lo:lo + 2 * LN_BLOCK, cols].astype(F32) - _after(mean, tok)
                part = jnp.sum((cen * cen).reshape(-1, 8, T), axis=0)
                sq = part if sq is None else sq + part
            var = jnp.sum(sq, axis=0, keepdims=True) / D
            inv = 1.0 / _round(jnp.sqrt(_round(_round(var) + EPS)))
            r = None
            for lo in range(0, D, LN_BLOCK):
                tok = yield
                rows = slice(lo, lo + LN_BLOCK)
                y = _round(xs[s, rows, cols].astype(F32) - _after(_round(mean), tok)) * inv
                y = y.astype(BF16)
                xn[s * NT + c, rows, :] = y
                part = jnp.sum((y.astype(F32) * wrb[rows, :]).reshape(-1, 8, T), axis=0)
                r = part if r is None else r + part
            rr[s, :, cols] = jnp.broadcast_to(jnp.sum(r, axis=0, keepdims=True), (8, T))

    def layernorm_now(tiles):
        start_background(layernorm(0, tiles))
        drain()

    def transpose_weights(src, dst):
        for lo, hi in CHUNKS:
            dst[lo // 2:hi // 2, :] = pltpu.bitcast(src[:, lo:hi].T, U32)

    def project(wt, rhs_of, consume, paced=0, sync=(), blocks=BLOCKS):
        for c, lo, hi in blocks:
            out = _dot(pltpu.bitcast(wt[lo // 2:hi // 2, :], BF16), rhs_of(c))
            if (c, lo) in sync:
                sync[c, lo]()
            flush()

            def post(c=c, lo=lo, hi=hi, out=out):
                consume(slice(c * T, (c + 1) * T), slice(lo, hi), out)
                for n in range(1, paced + 1):
                    row = n * (hi - lo) // paced
                    pace(out[row - 1:row])

            deferred.append(post)

    def keys(s, **kw):
        kt[s, D:, :] = jnp.zeros((_win(NG - 1) + T - D, L), BF16)

        def consume(cols, rows, k):
            kt[s, rows, cols] = k.astype(BF16)
            if s + 1 < NSEG:
                pk[s, rows, cols] = _phi(k).astype(BF16)
            if rows.stop == D and cols.stop % (2 * T) == 0:
                t0 = cols.stop - 2 * T
                for g in range(NG):
                    kg[s, g, t0 // 2:t0 // 2 + T, :] = pltpu.bitcast(
                        kt[s, _win(g):_win(g) + T, t0:t0 + 2 * T].T, U32)

        project(wkt, lambda c: xn[s * NT + c], consume, **kw)

    def queries(s, **kw):
        def consume(cols, rows, q):
            qt[s, rows.start // 2:rows.stop // 2, cols] = pltpu.bitcast(
                (q * QSCALE).astype(BF16), U32)
            if s > 0:
                pq[s, rows, cols] = _phi(q).astype(BF16)

        project(wqt, lambda c: xn[s * NT + c], consume, **kw)

    def vals(s, **kw):
        def consume(cols, rows, v):
            vt[s, rows, cols] = _round(v)

        project(wvt, lambda c: xn[s * NT + c], consume, **kw)

    mem = {}
    own = []
    for off in (0, 8):
        row = _iota((GW, GW), 0)
        col_head = _head_of(_iota((GW, GW), 1) - off)
        own.append((jnp.where(row < GF, _head_of(row), row - GF) == col_head) & (row < GF + 4))

    def remember(s):
        for g in range(NG):
            lhs = jnp.concatenate([vt[s, GF * g:GF * (g + 1), :], jnp.ones((8, L), F32)], axis=0)
            upd = _dot(lhs, pk[s, _win(g):_win(g) + GW, :], 1, 1)
            mem[g] = upd if s == 0 else mem[g] + upd
            flush()

    def recall(s):
        for g in range(NG):
            lhs = jnp.where(own[g % 2], mem[g], 0.0)
            g4 = gate[8 * (g // 2):8 * (g // 2) + 8, :]
            if g % 2:
                g4 = pltpu.roll(g4, 4, 0)
            for c in range(NT):
                cols = slice(c * T, (c + 1) * T)
                a = _dot(lhs, pq[s, _win(g):_win(g) + GW, cols])
                ot[s, GF * g:GF * (g + 1), cols] = a[0:GF] * _spread(g4 / (a[GF:GW] + 1e-6))
            flush()

    picked = []

    def route():
        tok = yield
        r = _after(_round(rr[...]), tok[:, 0:1])
        pos = (_iota(r.shape, 0) * L + _iota(r.shape, 2)).astype(F32)

        def top(scores, allowed):
            best = jnp.max(scores)
            return best, jnp.min(jnp.where((scores == best) & allowed, pos, float(S - 1)))

        r0, p0 = top(r, pos >= 0.0)
        r1, p1 = top(jnp.where(pos == p0, -jnp.inf, r), pos != p0)
        i0 = jnp.clip(p0.astype(jnp.int32), 0, S - 1)
        i1 = jnp.clip(p1.astype(jnp.int32), 0, S - 1)
        picked.extend([(r0, i0), (r1, i1)])
        for s in range(NSEG):
            ot[s, D:DE, :] = _onehot(0, i0 - s * L, (16, L)) + _onehot(1, i1 - s * L, (16, L))

    def ffn():
        (r0, i0), (r1, i1) = picked
        x_sel = (_dot(_onehot(0, i0 % T, (8, T)), xn[i0 // T], 1, 1)
                 + _dot(_onehot(1, i1 % T, (8, T)), xn[i1 // T], 1, 1))
        for _ in range(12):
            yield
        hid, y = {}, {}

        def up(i):
            both = []
            for w in (wg, wu):
                part = None
                for lo, hi in CHUNKS:
                    t = _dot(x_sel[:, lo:hi], w[lo:hi, i * T:(i + 1) * T])
                    part = t if part is None else part + t
                    yield
                both.append(part)
            hid[i] = _round(both[0] * jax.nn.sigmoid(both[0]) * both[1])

        def down(i):
            for lo, hi in CHUNKS:
                t = _dot(hid[i], wd[lo:hi, i * T:(i + 1) * T], 1, 1)
                y[lo] = t if i == 0 else y[lo] + t
                yield

        n = FF // T
        for i in range(n + 2):
            if i < n:
                yield from up(i)
            if i >= 2:
                yield from down(i - 2)
        out = jnp.concatenate([y[lo] for lo, _ in CHUNKS], axis=1)
        out = out * jax.nn.sigmoid(jnp.where(_iota((8, D), 0) == 0, r0, r1))
        wo[D:DE, :] = jnp.concatenate([out, jnp.zeros((8, D), F32)], axis=0).astype(BF16)
        transpose_weights(wo, wot)

    def q_rows(s, h, j):
        lo, w0 = DH * h, _win(h // 4)
        parts = []
        for b in range(w0, w0 + T, 16):
            if b + 16 <= lo or b >= lo + DH:
                parts.append(None)
                continue
            u = qt[s, b // 2:b // 2 + 8, j * T:(j + 1) * T]
            row = _iota((8, T), 0) * 2 + b
            if not (lo <= b and b + 16 <= lo + DH):
                u = jnp.where((row >= lo) & (row < lo + DH), u, jnp.zeros_like(u))
            parts.append(pltpu.roll(u, B * (h % 4), 1) if h % 4 else u)
        return parts

    def weights(parts):
        return jnp.concatenate([jnp.zeros((16, T), BF16) if p is None else pltpu.bitcast(p, BF16)
                                for p in parts], axis=0)

    mx, prob, acc, head = {}, {}, {}, {}

    def running_max(s, h, j, c, m):
        mx[s, h, j, c] = m if c == 0 else jnp.maximum(m, mx[s, h, j, c - 1])
        return mx[s, h, j, c]

    def scores(s, g, j, c):
        def k_rows(lo, n):
            return pltpu.bitcast(kg[s, g, lo // 2:(lo + n) // 2, :], BF16)

        if c < j:
            for h in range(4 * g, 4 * g + 4):
                sc = _dot(k_rows(c * T, T + B * (c + 1 == j)), weights(q_rows(s, h, j)))
                if c + 1 == j:
                    sc, head[h, j] = sc[:T], sc[T:]
                m = running_max(s, h, j, c, jnp.max(sc, axis=0, keepdims=True))
                prob[s, h, j, c] = jnp.exp2(sc - m).astype(BF16)
            return
        q = [q_rows(s, 4 * g + a, j) for a in range(4)]
        sc, top = [], []
        for n, (kb, heads) in enumerate(PASSES):
            if kb == 0 and j > 0:
                sc.append(head[4 * g + n, j] + mask[n])
            else:
                parts = [None if all(q[a][i] is None for a in heads)
                         else _by_block([q[a][i] for a in heads]) for i in range(T // 16)]
                sc.append(_dot(k_rows(c * T + kb * B, B), weights(parts)) + mask[n])
            top.append(jnp.max(sc[n].reshape(B // 8, 8, T), axis=0))

        def gather(a, kb, per_pass, fill):
            src = [fill] * NB
            for n, (k, heads) in enumerate(PASSES):
                for p in range(NB):
                    if k == kb and heads[p] == a:
                        src[p] = per_pass[n]
            return _by_block(src)

        low = jnp.full((8, T), NEG, F32)
        m = []
        for a in range(4):
            t = gather(a, 0, top, low)
            for kb in range(1, NB):
                t = jnp.maximum(t, gather(a, kb, top, low))
            m.append(running_max(s, 4 * g + a, j, c, jnp.max(t, axis=0, keepdims=True)))
        e = [jnp.exp2(sc[n] - _by_block([m[a] for a in heads]))
             for n, (_, heads) in enumerate(PASSES)]
        for a in range(4):
            prob[s, 4 * g + a, j, c] = jnp.concatenate(
                [gather(a, kb, e, None) for kb in range(NB)], axis=0).astype(BF16)

    def values(s, g, j, c):
        done = []
        for h in range(4 * g, 4 * g + 4):
            v0 = (DH * h // 8) * 8
            ones = 0 if DH * h > v0 else 23
            v = vt[s, v0:v0 + 24, c * T:(c + 1) * T]
            v = jnp.where(_iota((24, T), 0) == ones, 1.0, v)
            o = _dot(v, prob.pop((s, h, j, c)))
            if c > 0:
                o = acc[h, j] * jnp.exp2(mx[s, h, j, c - 1] - mx[s, h, j, c]) + o
            acc[h, j] = o
            if c == j:
                o = o * ((1.0 - gate[h:h + 1, :]) / o[ones:ones + 1, :])
                done.append(pltpu.roll(o, T - B * (h % 4), 1) if h % 4 else o)
        if c == j:
            sub = _iota((8, T), 0)
            rows = [done[0][0:16]]
            for i in range(1, 4):
                rows.append(jnp.where(sub < 2 * i, done[i - 1][16:24], done[i][0:8]))
                rows.append(done[i][8:16])
            rows.append(done[3][16:24])
            o = jnp.concatenate(rows, axis=0)
            at = (s, slice(GF * g, GF * (g + 1)), slice(j * T, (j + 1) * T))
            ot[at] = o if s == 0 else ot[at] + o

    def attention(segs, hook):
        steps = [(s, g, j, c) for s in segs for g in range(NG) for j, c in TILES]
        for i in range(len(steps)):
            scores(*steps[i])
            flush()
            if i >= PV_DELAY:
                s, g, j, c = steps[i - PV_DELAY]
                values(s, g, j, c)
                hook(i - PV_DELAY, mx[s, 4 * g, j, c])
        later.extend(lambda step=step: values(*step) for step in steps[-PV_DELAY:])

    def finish(s):
        blocks, sends = BLOCKS, {(NT - 1, D): (0, D, 0, L)}
        if s == 0:
            blocks = sorted(BLOCKS, key=lambda b: b[1])
        if s == NSEG - 1:
            blocks = BLOCKS[:-1] + ((NT - 1, D - MC, D - MC // 2), (NT - 1, D - MC // 2, D))
            sends = {(NT - 2, D): (0, D, 0, L - T), (NT - 1, D - MC): (0, D - MC, L - T, L),
                     (NT - 1, D): (D - MC, D, L - T, L)}

        def consume(cols, rows, o):
            c = cols.start // T
            res = xs[s, rows, cols].astype(F32) + xn[s * NT + c, rows, :].astype(F32)
            outb[s, rows, cols] = (o + res).astype(BF16)
            if (c, rows.stop) in sends:
                send(s, *sends[c, rows.stop])

        project(wot, lambda c: ot[s, :, c * T:(c + 1) * T].astype(BF16), consume, blocks=blocks)

    x_head.wait()
    layernorm_now((0, 1))
    c_wq.start()
    c_wv.start()
    c_wk.wait()
    transpose_weights(wk, wkt)
    near_end = (NT - 1, MC)
    keys(0, sync={(1, 0): wave([x_tail], (), lambda: layernorm_now((2, 3))),
                  near_end: wave([c_wq], x_rest, lambda: transpose_weights(wq, wqt))})
    queries(0, sync={near_end: wave([c_wv], (), lambda: transpose_weights(wv, wvt))})
    vals(0, sync={near_end: wave(x_rest, late)})
    start_background(layernorm(1))
    attention([0], lambda i, token: pace(token) if i % 3 == 0 else None)
    drain()
    for s in range(1, NSEG):
        more = s + 1 < NSEG
        keys(s)
        remember(s - 1)
        queries(s)
        flush()
        recall(s)
        start_background(layernorm(s + 1) if more else route())
        vals(s, paced=2, sync=() if more else {near_end: wave(late)})
        if more:
            flush()
            drain()

    routed = ffn()

    def ffn_steps(i, token):
        for _ in range(FFN_RATE[i % len(FFN_RATE)]):
            next(routed, None)

    attention(range(1, NSEG), ffn_steps)
    for _ in routed:
        pass
    for s in range(NSEG):
        finish(s)
    flush()
    for c in out_copies:
        c.wait()


@jax.jit
def pallas_parallel_sum__memory_aug_infini_attn__moe_arch_mod__prompt_kernel(
    A_x: jax.Array,
    A_wq: jax.Array,
    A_wk: jax.Array,
    A_wv: jax.Array,
    A_wo: jax.Array,
    A_beta: jax.Array,
    B_x: jax.Array,
    B_w_r: jax.Array,
    B_w_gate: jax.Array,
    B_w_up: jax.Array,
    B_w_down: jax.Array,
):
    del B_x
    scratch = [
        pltpu.VMEM((NSEG, D, L), BF16),
        pltpu.VMEM((NSEG * NT, D, T), BF16),
        pltpu.VMEM((D, D), BF16),
        pltpu.VMEM((D, D), BF16),
        pltpu.VMEM((D, D), BF16),
        pltpu.VMEM((DE, D), BF16),
        pltpu.VMEM((H,), BF16),
        pltpu.VMEM((D,), BF16),
        pltpu.VMEM((D, FF), BF16),
        pltpu.VMEM((D, FF), BF16),
        pltpu.VMEM((D, FF), BF16),
        pltpu.VMEM((D // 2, D), U32),
        pltpu.VMEM((D // 2, D), U32),
        pltpu.VMEM((D // 2, D), U32),
        pltpu.VMEM((D // 2, DE), U32),
        pltpu.VMEM((NSEG, D // 2, L), U32),
        pltpu.VMEM((NSEG, D, L), BF16),
        pltpu.VMEM((NSEG, D, L), BF16),
        pltpu.VMEM((NSEG, D, L), F32),
        pltpu.VMEM((NSEG, _win(NG - 1) + T, L), BF16),
        pltpu.VMEM((NSEG, NG, L // 2, T), U32),
        pltpu.VMEM((NSEG, DE, L), F32),
        pltpu.VMEM((NSEG, 8, L), F32),
        pltpu.VMEM((D, T), F32),
        pltpu.VMEM((H, T), F32),
        pltpu.VMEM((len(PASSES), B, T), F32),
        pltpu.VMEM((NSEG, D, L), BF16),
        pltpu.SemaphoreType.DMA((NSEG + 1,)),
        pltpu.SemaphoreType.DMA((9,)),
        pltpu.SemaphoreType.DMA((NSEG + 2,)),
    ]
    out_t = pl.pallas_call(
        _kernel,
        out_shape=jax.ShapeDtypeStruct((D, S), BF16),
        in_specs=[pl.BlockSpec(memory_space=pl.ANY)] * 10,
        out_specs=pl.BlockSpec(memory_space=pl.ANY),
        scratch_shapes=scratch,
        compiler_params=pltpu.CompilerParams(vmem_limit_bytes=100 * 1024 * 1024),
        name="infini_mod",
    )(A_x.reshape(S, D).T, A_wq, A_wk, A_wv, A_wo, A_beta, B_w_r, B_w_gate, B_w_up, B_w_down.T)
    return out_t.T.reshape(1, S, D)
```

```python
import jax
import jax.numpy as jnp
import numpy as np
from jax import lax
import jax.experimental.pallas as pl
import jax.experimental.pallas.tpu as pltpu

F32, BF16, U32 = jnp.float32, jnp.bfloat16, jnp.uint32

S, D, H, NSEG, FF = 2048, 576, 32, 4, 4608
DH = D // H
L = S // NSEG
T = 128
NT = L // T
NG = H // 4
GF = 4 * DH
GW = 80
DE = D + 16
QSCALE = float(DH ** -0.5 * np.log2(np.e))
EPS = float(np.asarray(1e-5, dtype=jnp.bfloat16))
NEG = -1e30
CHUNKS = ((0, 128), (128, 256), (256, 384), (384, 512), (512, 576))
MC = 192
BLOCKS = tuple((c, lo, lo + MC) for c in range(NT) for lo in range(0, D, MC))
LN_BLOCK = 144

TILES = ((3, 0), (0, 0), (3, 1), (3, 2), (3, 3), (1, 0), (1, 1), (2, 0), (2, 1), (2, 2))
FFN_RATE = (4, 4, 0, 4, 0, 4, 4, 0, 4, 0)
PV_DELAY = 2
NB = 4
B = T // NB
PASSES = (
    (0, (0, 0, 0, 0)), (0, (1, 1, 1, 1)), (0, (2, 2, 2, 2)), (0, (3, 3, 3, 3)),
    (1, (3, 0, 0, 0)), (1, (1, 3, 1, 1)), (1, (2, 2, 3, 2)),
    (2, (2, 2, 0, 0)), (2, (1, 3, 3, 1)),
    (3, (1, 2, 3, 0)),
)


def _dot(a, b, ca=1, cb=0):
    return lax.dot_general(a, b, (((ca,), (cb,)), ((), ())), preferred_element_type=F32)


def _iota(shape, dim):
    return lax.broadcasted_iota(jnp.int32, shape, dim)


def _round(x):
    return x.astype(BF16).astype(F32)


def _phi(t):
    return jnp.where(t > 0, t + 1.0, jnp.exp(t))


def _win(g):
    return (GF * g // 16) * 16


def _after(value, token):
    if token is None:
        return value
    return jnp.where(token * token < 0.0, 0.0, value)


def _onehot(row, lane, shape):
    return jnp.where((_iota(shape, 0) == row) & (_iota(shape, 1) == lane), 1.0, 0.0)


def _head_of(d):
    h = jnp.full(d.shape, -1, jnp.int32)
    for i in range(5):
        h = jnp.where(d >= i * DH, i, h)
    return h


def _spread(rows):
    sub = _iota(rows.shape, 0)
    full = [jnp.broadcast_to(rows[i:i + 1], rows.shape) for i in range(4)]
    out = []
    for v in range(GF // 8):
        a, b = 8 * v // DH, (8 * v + 7) // DH
        out.append(full[a] if a == b else jnp.where(sub < DH * b - 8 * v, full[a], full[b]))
    return jnp.concatenate(out, axis=0)


def _kernel(x_hbm, wq_hbm, wk_hbm, wv_hbm, wo_hbm, beta_hbm, wr_hbm, wg_hbm, wu_hbm, wd_hbm,
            out_hbm,
            xs, xn, wq, wk, wv, wo, beta, wr, wg, wu, wd,
            wqt, wkt, wvt, wot, qt, pq, pk, vt, kt, kg, ot, rr, wrb, gate, mask, outb,
            sem_x, sem_w, sem_o):
    def x_copy(s, lo, hi, sem):
        return pltpu.make_async_copy(x_hbm.at[:, pl.ds(s * L + lo, hi - lo)],
                                     xs.at[s, :, pl.ds(lo, hi - lo)], sem_x.at[sem])

    x_head, x_tail = x_copy(0, 0, L // 2, 0), x_copy(0, L // 2, L, 1)
    x_rest = [x_copy(s, 0, L, s + 1) for s in range(1, NSEG)]
    c_wr, c_beta, c_wq, c_wk, c_wv, *late = [
        pltpu.make_async_copy(src, dst, sem_w.at[i]) for i, (src, dst) in enumerate((
            (wr_hbm, wr), (beta_hbm, beta), (wq_hbm, wq), (wk_hbm, wk), (wv_hbm, wv),
            (wg_hbm, wg), (wu_hbm, wu), (wd_hbm, wd), (wo_hbm, wo.at[pl.ds(0, D)])))]
    out_copies = []

    def send(s, r0, r1, c0, c1):
        c = pltpu.make_async_copy(outb.at[s, pl.ds(r0, r1 - r0), pl.ds(c0, c1 - c0)],
                                  out_hbm.at[pl.ds(r0, r1 - r0), pl.ds(s * L + c0, c1 - c0)],
                                  sem_o.at[len(out_copies)])
        c.start()
        out_copies.append(c)

    def wave(wait, start=(), then=None):
        def sync():
            for c in start:
                c.start()
            for c in wait:
                c.wait()
            if then is not None:
                then()
        return sync

    for c in (c_wr, c_beta, x_head, c_wk, x_tail):
        c.start()

    memo = {}

    def once(name, make):
        if name not in memo:
            memo[name] = make()
        return memo[name]

    def by_block(vals):
        ref = next(v for v in vals if v is not None)
        groups = []
        for p, v in enumerate(vals):
            for got, ps in groups:
                if got is v:
                    ps.append(p)
                    break
            else:
                groups.append((v, [p]))
        groups.sort(key=lambda e: -len(e[1]))
        out = None
        for v, ps in groups:
            if v is None:
                v = once(("zero", ref.shape, ref.dtype), lambda: jnp.zeros_like(ref))
            if out is None:
                out = v
                continue
            bits = sum(1 << p for p in ps)
            hit = once(("blocks", ref.shape, bits),
                       lambda: ((bits >> (_iota(ref.shape, 1) // B)) & 1) == 1)
            out = jnp.where(hit, v, out)
        return out

    key, lane = _iota((B, T), 0), _iota((B, T), 1)
    for n, (kb, heads) in enumerate(PASSES):
        shift = by_block([jnp.full((B, T), ((p - a) % NB - p) * B) for p, a in enumerate(heads)])
        mask[n] = jnp.where(key + kb * B <= lane + shift, 0.0, NEG)
    c_wr.wait()
    c_beta.wait()
    wrb[...] = jnp.broadcast_to(wr[...].astype(F32).reshape(1, D), (T, D)).T
    g_row = jax.nn.sigmoid(beta[...].astype(F32).reshape(1, H))
    gate[...] = jnp.broadcast_to(g_row, (T, H)).T

    background = []
    deferred = []
    later = []

    def start_background(gen):
        next(gen)
        background.append(gen)

    def pace(token):
        if background:
            try:
                background[0].send(token)
            except StopIteration:
                background.pop(0)

    def drain():
        while background:
            pace(None)

    def flush():
        while deferred:
            deferred.pop(0)()
        if later:
            later.pop(0)()

    def layernorm(s, tiles=range(NT)):
        for c in tiles:
            cols = slice(c * T, (c + 1) * T)
            mean = jnp.sum(xs[s, :, cols].astype(F32), axis=0, keepdims=True) / D
            sq = None
            for lo in range(0, D, 2 * LN_BLOCK):
                tok = yield
                cen = xs[s, lo:lo + 2 * LN_BLOCK, cols].astype(F32) - _after(mean, tok)
                part = jnp.sum((cen * cen).reshape(-1, 8, T), axis=0)
                sq = part if sq is None else sq + part
            var = jnp.sum(sq, axis=0, keepdims=True) / D
            inv = 1.0 / _round(jnp.sqrt(_round(_round(var) + EPS)))
            r = None
            for lo in range(0, D, LN_BLOCK):
                tok = yield
                rows = slice(lo, lo + LN_BLOCK)
                y = _round(xs[s, rows, cols].astype(F32) - _after(_round(mean), tok)) * inv
                y = y.astype(BF16)
                xn[s * NT + c, rows, :] = y
                part = jnp.sum((y.astype(F32) * wrb[rows, :]).reshape(-1, 8, T), axis=0)
                r = part if r is None else r + part
            rr[s, :, cols] = jnp.broadcast_to(jnp.sum(r, axis=0, keepdims=True), (8, T))

    def layernorm_now(tiles):
        start_background(layernorm(0, tiles))
        drain()

    def transpose_weights(src, dst):
        for lo, hi in CHUNKS:
            dst[lo // 2:hi // 2, :] = pltpu.bitcast(src[:, lo:hi].T, U32)

    def project(wt, rhs_of, consume, paced=0, sync=(), blocks=BLOCKS):
        for c, lo, hi in blocks:
            out = _dot(pltpu.bitcast(wt[lo // 2:hi // 2, :], BF16), rhs_of(c))
            if (c, lo) in sync:
                sync[c, lo]()
            flush()

            def post(c=c, lo=lo, hi=hi, out=out):
                consume(slice(c * T, (c + 1) * T), slice(lo, hi), out)
                for n in range(1, paced + 1):
                    row = n * (hi - lo) // paced
                    pace(out[row - 1:row])

            deferred.append(post)

    def keys(s, **kw):
        kt[s, D:, :] = jnp.zeros((_win(NG - 1) + T - D, L), BF16)

        def consume(cols, rows, k):
            kt[s, rows, cols] = k.astype(BF16)
            if s + 1 < NSEG:
                pk[s, rows, cols] = _phi(k).astype(BF16)
            if rows.stop == D and cols.stop % (2 * T) == 0:
                t0 = cols.stop - 2 * T
                for g in range(NG):
                    kg[s, g, t0 // 2:t0 // 2 + T, :] = pltpu.bitcast(
                        kt[s, _win(g):_win(g) + T, t0:t0 + 2 * T].T, U32)

        project(wkt, lambda c: xn[s * NT + c], consume, **kw)

    def queries(s, **kw):
        def consume(cols, rows, q):
            qt[s, rows.start // 2:rows.stop // 2, cols] = pltpu.bitcast(
                (q * QSCALE).astype(BF16), U32)
            if s > 0:
                pq[s, rows, cols] = _phi(q).astype(BF16)

        project(wqt, lambda c: xn[s * NT + c], consume, **kw)

    def vals(s, **kw):
        def consume(cols, rows, v):
            vt[s, rows, cols] = _round(v)

        project(wvt, lambda c: xn[s * NT + c], consume, **kw)

    mem = {}
    own = []
    for off in (0, 8):
        row = _iota((GW, GW), 0)
        col_head = _head_of(_iota((GW, GW), 1) - off)
        own.append((jnp.where(row < GF, _head_of(row), row - GF) == col_head) & (row < GF + 4))

    def remember(s):
        for g in range(NG):
            lhs = jnp.concatenate([vt[s, GF * g:GF * (g + 1), :], jnp.ones((8, L), F32)], axis=0)
            upd = _dot(lhs, pk[s, _win(g):_win(g) + GW, :], 1, 1)
            mem[g] = upd if s == 0 else mem[g] + upd
            flush()

    def recall(s):
        for g in range(NG):
            lhs = jnp.where(own[g % 2], mem[g], 0.0)
            g4 = gate[8 * (g // 2):8 * (g // 2) + 8, :]
            if g % 2:
                g4 = pltpu.roll(g4, 4, 0)
            for c in range(NT):
                cols = slice(c * T, (c + 1) * T)
                a = _dot(lhs, pq[s, _win(g):_win(g) + GW, cols])
                ot[s, GF * g:GF * (g + 1), cols] = a[0:GF] * _spread(g4 / (a[GF:GW] + 1e-6))
            flush()

    picked = []

    def route():
        tok = yield
        r = _after(_round(rr[...]), tok[:, 0:1])
        pos = (_iota(r.shape, 0) * L + _iota(r.shape, 2)).astype(F32)

        def top(scores, allowed):
            best = jnp.max(scores)
            return best, jnp.min(jnp.where((scores == best) & allowed, pos, float(S - 1)))

        r0, p0 = top(r, pos >= 0.0)
        r1, p1 = top(jnp.where(pos == p0, -jnp.inf, r), pos != p0)
        i0 = jnp.clip(p0.astype(jnp.int32), 0, S - 1)
        i1 = jnp.clip(p1.astype(jnp.int32), 0, S - 1)
        picked.extend([(r0, i0), (r1, i1)])
        for s in range(NSEG):
            ot[s, D:DE, :] = _onehot(0, i0 - s * L, (16, L)) + _onehot(1, i1 - s * L, (16, L))

    def ffn():
        (r0, i0), (r1, i1) = picked
        x_sel = (_dot(_onehot(0, i0 % T, (8, T)), xn[i0 // T], 1, 1)
                 + _dot(_onehot(1, i1 % T, (8, T)), xn[i1 // T], 1, 1))
        for _ in range(12):
            yield
        hid, y = {}, {}

        def up(i):
            both = []
            for w in (wg, wu):
                part = None
                for lo, hi in CHUNKS:
                    t = _dot(x_sel[:, lo:hi], w[lo:hi, i * T:(i + 1) * T])
                    part = t if part is None else part + t
                    yield
                both.append(part)
            hid[i] = _round(both[0] * jax.nn.sigmoid(both[0]) * both[1])

        def down(i):
            for lo, hi in CHUNKS:
                t = _dot(hid[i], wd[lo:hi, i * T:(i + 1) * T], 1, 1)
                y[lo] = t if i == 0 else y[lo] + t
                yield

        n = FF // T
        for i in range(n + 2):
            if i < n:
                yield from up(i)
            if i >= 2:
                yield from down(i - 2)
        out = jnp.concatenate([y[lo] for lo, _ in CHUNKS], axis=1)
        out = out * jax.nn.sigmoid(jnp.where(_iota((8, D), 0) == 0, r0, r1))
        wo[D:DE, :] = jnp.concatenate([out, jnp.zeros((8, D), F32)], axis=0).astype(BF16)
        transpose_weights(wo, wot)

    def q_rows(s, h, j):
        lo, w0 = DH * h, _win(h // 4)
        parts = []
        for b in range(w0, w0 + T, 16):
            if b + 16 <= lo or b >= lo + DH:
                parts.append(None)
                continue
            u = qt[s, b // 2:b // 2 + 8, j * T:(j + 1) * T]
            if not (lo <= b and b + 16 <= lo + DH):
                row = once("row", lambda: _iota((8, T), 0) * 2)
                keep = once(("rows", lo - b), lambda: (row >= lo - b) & (row < lo - b + DH))
                u = jnp.where(keep, u, jnp.zeros_like(u))
            parts.append(pltpu.roll(u, B * (h % 4), 1) if h % 4 else u)
        return parts

    def weights(parts):
        zero = once("zero", lambda: jnp.zeros((16, T), BF16))
        return jnp.concatenate(
            [zero if p is None else pltpu.bitcast(p, BF16) for p in parts], axis=0)

    mx, prob, acc, head = {}, {}, {}, {}

    def running_max(s, h, j, c, m):
        mx[s, h, j, c] = m if c == 0 else jnp.maximum(m, mx[s, h, j, c - 1])
        return mx[s, h, j, c]

    def scores(s, g, j, c):
        def k_rows(lo, n):
            return pltpu.bitcast(kg[s, g, lo // 2:(lo + n) // 2, :], BF16)

        if c < j:
            for h in range(4 * g, 4 * g + 4):
                sc = _dot(k_rows(c * T, T + B * (c + 1 == j)), weights(once((s, h, j), lambda: q_rows(s, h, j))))
                if c + 1 == j:
                    sc, head[h, j] = sc[:T], sc[T:]
                m = running_max(s, h, j, c, jnp.max(sc, axis=0, keepdims=True))
                prob[s, h, j, c] = jnp.exp2(sc - m).astype(BF16)
            return
        q = [once((s, h, j), lambda: q_rows(s, h, j)) for h in range(4 * g, 4 * g + 4)]
        sc, top = [], []
        for n, (kb, heads) in enumerate(PASSES):
            if kb == 0 and j > 0:
                sc.append(head[4 * g + n, j] + mask[n])
            else:
                parts = [None if all(q[a][i] is None for a in heads)
                         else by_block([q[a][i] for a in heads]) for i in range(T // 16)]
                sc.append(_dot(k_rows(c * T + kb * B, B), weights(parts)) + mask[n])
            top.append(jnp.max(sc[n].reshape(B // 8, 8, T), axis=0))

        def gather(a, kb, per_pass, fill):
            src = [fill] * NB
            for n, (k, heads) in enumerate(PASSES):
                for p in range(NB):
                    if k == kb and heads[p] == a:
                        src[p] = per_pass[n]
            return by_block(src)

        low = jnp.full((8, T), NEG, F32)
        m = []
        for a in range(4):
            t = gather(a, 0, top, low)
            for kb in range(1, NB):
                t = jnp.maximum(t, gather(a, kb, top, low))
            m.append(running_max(s, 4 * g + a, j, c, jnp.max(t, axis=0, keepdims=True)))
        e = [jnp.exp2(sc[n] - by_block([m[a] for a in heads]))
             for n, (_, heads) in enumerate(PASSES)]
        for a in range(4):
            prob[s, 4 * g + a, j, c] = jnp.concatenate(
                [gather(a, kb, e, None) for kb in range(NB)], axis=0).astype(BF16)

    def values(s, g, j, c):
        done = []
        for h in range(4 * g, 4 * g + 4):
            v0 = (DH * h // 8) * 8
            ones = 0 if DH * h > v0 else 23
            v = vt[s, v0:v0 + 24, c * T:(c + 1) * T]
            v = jnp.where(once(("ones", ones), lambda: _iota((24, T), 0) == ones), 1.0, v)
            o = _dot(v, prob.pop((s, h, j, c)))
            if c > 0:
                o = acc[h, j] * jnp.exp2(mx[s, h, j, c - 1] - mx[s, h, j, c]) + o
            acc[h, j] = o
            if c == j:
                o = o * ((1.0 - gate[h:h + 1, :]) / o[ones:ones + 1, :])
                done.append(pltpu.roll(o, T - B * (h % 4), 1) if h % 4 else o)
        if c == j:
            sub = _iota((8, T), 0)
            rows = [done[0][0:16]]
            for i in range(1, 4):
                rows.append(jnp.where(sub < 2 * i, done[i - 1][16:24], done[i][0:8]))
                rows.append(done[i][8:16])
            rows.append(done[3][16:24])
            o = jnp.concatenate(rows, axis=0)
            at = (s, slice(GF * g, GF * (g + 1)), slice(j * T, (j + 1) * T))
            ot[at] = o if s == 0 else ot[at] + o

    def attention(segs, hook):
        steps = [(s, g, j, c) for s in segs for g in range(NG) for j, c in TILES]
        for i in range(len(steps)):
            scores(*steps[i])
            flush()
            if i >= PV_DELAY:
                s, g, j, c = steps[i - PV_DELAY]
                values(s, g, j, c)
                hook(i - PV_DELAY, mx[s, 4 * g, j, c])
        later.extend(lambda step=step: values(*step) for step in steps[-PV_DELAY:])

    def finish(s):
        blocks, sends = BLOCKS, {(NT - 1, D): (0, D, 0, L)}
        if s == 0:
            blocks = sorted(BLOCKS, key=lambda b: b[1])
        if s == NSEG - 1:
            blocks = BLOCKS[:-1] + ((NT - 1, D - MC, D - MC // 2), (NT - 1, D - MC // 2, D))
            sends = {(NT - 2, D): (0, D, 0, L - T), (NT - 1, D - MC): (0, D - MC, L - T, L),
                     (NT - 1, D): (D - MC, D, L - T, L)}

        def consume(cols, rows, o):
            c = cols.start // T
            res = xs[s, rows, cols].astype(F32) + xn[s * NT + c, rows, :].astype(F32)
            outb[s, rows, cols] = (o + res).astype(BF16)
            if (c, rows.stop) in sends:
                send(s, *sends[c, rows.stop])

        project(wot, lambda c: ot[s, :, c * T:(c + 1) * T].astype(BF16), consume, blocks=blocks)

    x_head.wait()
    layernorm_now((0, 1))
    c_wq.start()
    c_wv.start()
    c_wk.wait()
    transpose_weights(wk, wkt)
    near_end = (NT - 1, MC)
    keys(0, sync={(1, 0): wave([x_tail], (), lambda: layernorm_now((2, 3))),
                  near_end: wave([c_wq], x_rest, lambda: transpose_weights(wq, wqt))})
    queries(0, sync={near_end: wave([c_wv], (), lambda: transpose_weights(wv, wvt))})
    vals(0, sync={near_end: wave(x_rest, late)})
    start_background(layernorm(1))
    attention([0], lambda i, token: pace(token) if i % 10 in (0, 3, 6) else None)
    drain()
    for s in range(1, NSEG):
        more = s + 1 < NSEG
        keys(s)
        remember(s - 1)
        queries(s)
        flush()
        recall(s)
        start_background(layernorm(s + 1) if more else route())
        vals(s, paced=2, sync=() if more else {near_end: wave(late)})
        if more:
            flush()
            drain()

    routed = ffn()

    def ffn_steps(i, token):
        for _ in range(FFN_RATE[i % len(FFN_RATE)]):
            next(routed, None)

    attention(range(1, NSEG), ffn_steps)
    for _ in routed:
        pass
    for s in range(NSEG):
        finish(s)
    flush()
    for c in out_copies:
        c.wait()


@jax.jit
def pallas_parallel_sum__memory_aug_infini_attn__moe_arch_mod__prompt_kernel(
    A_x: jax.Array,
    A_wq: jax.Array,
    A_wk: jax.Array,
    A_wv: jax.Array,
    A_wo: jax.Array,
    A_beta: jax.Array,
    B_x: jax.Array,
    B_w_r: jax.Array,
    B_w_gate: jax.Array,
    B_w_up: jax.Array,
    B_w_down: jax.Array,
):
    del B_x
    scratch = [
        pltpu.VMEM((NSEG, D, L), BF16),
        pltpu.VMEM((NSEG * NT, D, T), BF16),
        pltpu.VMEM((D, D), BF16),
        pltpu.VMEM((D, D), BF16),
        pltpu.VMEM((D, D), BF16),
        pltpu.VMEM((DE, D), BF16),
        pltpu.VMEM((H,), BF16),
        pltpu.VMEM((D,), BF16),
        pltpu.VMEM((D, FF), BF16),
        pltpu.VMEM((D, FF), BF16),
        pltpu.VMEM((D, FF), BF16),
        pltpu.VMEM((D // 2, D), U32),
        pltpu.VMEM((D // 2, D), U32),
        pltpu.VMEM((D // 2, D), U32),
        pltpu.VMEM((D // 2, DE), U32),
        pltpu.VMEM((NSEG, D // 2, L), U32),
        pltpu.VMEM((NSEG, D, L), BF16),
        pltpu.VMEM((NSEG, D, L), BF16),
        pltpu.VMEM((NSEG, D, L), F32),
        pltpu.VMEM((NSEG, _win(NG - 1) + T, L), BF16),
        pltpu.VMEM((NSEG, NG, L // 2, T), U32),
        pltpu.VMEM((NSEG, DE, L), F32),
        pltpu.VMEM((NSEG, 8, L), F32),
        pltpu.VMEM((D, T), F32),
        pltpu.VMEM((H, T), F32),
        pltpu.VMEM((len(PASSES), B, T), F32),
        pltpu.VMEM((NSEG, D, L), BF16),
        pltpu.SemaphoreType.DMA((NSEG + 1,)),
        pltpu.SemaphoreType.DMA((9,)),
        pltpu.SemaphoreType.DMA((NSEG + 2,)),
    ]
    out_t = pl.pallas_call(
        _kernel,
        out_shape=jax.ShapeDtypeStruct((D, S), BF16),
        in_specs=[pl.BlockSpec(memory_space=pl.ANY)] * 10,
        out_specs=pl.BlockSpec(memory_space=pl.ANY),
        scratch_shapes=scratch,
        compiler_params=pltpu.CompilerParams(vmem_limit_bytes=100 * 1024 * 1024),
        name="infini_mod",
    )(A_x.reshape(S, D).T, A_wq, A_wk, A_wv, A_wo, A_beta, B_w_r, B_w_gate, B_w_up, B_w_down.T)
    return out_t.T.reshape(1, S, D)
```

```python
import jax
import jax.numpy as jnp
import numpy as np
from jax import lax
import jax.experimental.pallas as pl
import jax.experimental.pallas.tpu as pltpu

F32, BF16, U32 = jnp.float32, jnp.bfloat16, jnp.uint32

S, D, H, NSEG, FF = 2048, 576, 32, 4, 4608
DH = D // H
L = S // NSEG
T = 128
NT = L // T
NG = H // 4
GF = 4 * DH
GW = 80
DE = D + 16
QSCALE = float(DH ** -0.5 * np.log2(np.e))
EPS = float(np.asarray(1e-5, dtype=jnp.bfloat16))
NEG = -1e30
CHUNKS = ((0, 128), (128, 256), (256, 384), (384, 512), (512, 576))
MC = 192
BLOCKS = tuple((c, lo, lo + MC) for c in range(NT) for lo in range(0, D, MC))
LN_BLOCK = 144

TILES = ((3, 0), (0, 0), (3, 1), (3, 2), (3, 3), (1, 0), (1, 1), (2, 0), (2, 1), (2, 2))
FFN_RATE = (4, 4, 0, 4, 0, 4, 4, 0, 4, 0)
PV_DELAY = 2
NB = 4
B = T // NB
PASSES = (
    (0, (0, 0, 0, 0)), (0, (1, 1, 1, 1)), (0, (2, 2, 2, 2)), (0, (3, 3, 3, 3)),
    (1, (3, 0, 0, 0)), (1, (1, 3, 1, 1)), (1, (2, 2, 3, 2)),
    (2, (2, 2, 0, 0)), (2, (1, 3, 3, 1)),
    (3, (1, 2, 3, 0)),
)


def _dot(a, b, ca=1, cb=0):
    return lax.dot_general(a, b, (((ca,), (cb,)), ((), ())), preferred_element_type=F32)


def _iota(shape, dim):
    return lax.broadcasted_iota(jnp.int32, shape, dim)


def _round(x):
    return x.astype(BF16).astype(F32)


def _phi(t):
    return jnp.where(t > 0, t + 1.0, jnp.exp(t))


def _win(g):
    return (GF * g // 16) * 16


def _after(value, token):
    if token is None:
        return value
    return jnp.where(token * token < 0.0, 0.0, value)


def _onehot(row, lane, shape):
    return jnp.where((_iota(shape, 0) == row) & (_iota(shape, 1) == lane), 1.0, 0.0)


def _head_of(d):
    h = jnp.full(d.shape, -1, jnp.int32)
    for i in range(5):
        h = jnp.where(d >= i * DH, i, h)
    return h


def _spread(rows):
    sub = _iota(rows.shape, 0)
    full = [jnp.broadcast_to(rows[i:i + 1], rows.shape) for i in range(4)]
    out = []
    for v in range(GF // 8):
        a, b = 8 * v // DH, (8 * v + 7) // DH
        out.append(full[a] if a == b else jnp.where(sub < DH * b - 8 * v, full[a], full[b]))
    return jnp.concatenate(out, axis=0)


def _kernel(x_hbm, wq_hbm, wk_hbm, wv_hbm, wo_hbm, beta_hbm, wr_hbm, wg_hbm, wu_hbm, wd_hbm,
            out_hbm,
            xs, xn, wq, wk, wv, wo, beta, wr, wg, wu, wd,
            wqt, wkt, wvt, wot, qt, pq, pk, vt, kt, kg, ot, rr, wrb, gate, mask, outb,
            sem_x, sem_w, sem_o):
    def x_copy(s, lo, hi, sem):
        return pltpu.make_async_copy(x_hbm.at[:, pl.ds(s * L + lo, hi - lo)],
                                     xs.at[s, :, pl.ds(lo, hi - lo)], sem_x.at[sem])

    x_head, x_tail = x_copy(0, 0, L // 2, 0), x_copy(0, L // 2, L, 1)
    x_rest = [x_copy(s, 0, L, s + 1) for s in range(1, NSEG)]
    left, right = pl.ds(0, 2 * T), pl.ds(2 * T, D - 2 * T)
    c_wr, c_beta, c_wq, wk_head, wk_tail, c_wv, *late = [
        pltpu.make_async_copy(src, dst, sem_w.at[i]) for i, (src, dst) in enumerate((
            (wr_hbm, wr), (beta_hbm, beta), (wq_hbm, wq),
            (wk_hbm.at[:, left], wk.at[:, left]), (wk_hbm.at[:, right], wk.at[:, right]),
            (wv_hbm, wv),
            (wg_hbm, wg), (wu_hbm, wu), (wd_hbm, wd), (wo_hbm, wo.at[pl.ds(0, D)])))]
    out_copies = []

    def send(s, r0, r1, c0, c1):
        c = pltpu.make_async_copy(outb.at[s, pl.ds(r0, r1 - r0), pl.ds(c0, c1 - c0)],
                                  out_hbm.at[pl.ds(r0, r1 - r0), pl.ds(s * L + c0, c1 - c0)],
                                  sem_o.at[len(out_copies)])
        c.start()
        out_copies.append(c)

    def wave(wait, start=(), then=None):
        def sync():
            for c in start:
                c.start()
            for c in wait:
                c.wait()
            if then is not None:
                then()
        return sync

    for c in (c_wr, c_beta, x_head, wk_head, x_tail, wk_tail):
        c.start()

    memo = {}

    def once(name, make):
        if name not in memo:
            memo[name] = make()
        return memo[name]

    def by_block(vals):
        ref = next(v for v in vals if v is not None)
        groups = []
        for p, v in enumerate(vals):
            for got, ps in groups:
                if got is v:
                    ps.append(p)
                    break
            else:
                groups.append((v, [p]))
        groups.sort(key=lambda e: -len(e[1]))
        out = None
        for v, ps in groups:
            if v is None:
                v = once(("zero", ref.shape, ref.dtype), lambda: jnp.zeros_like(ref))
            if out is None:
                out = v
                continue
            bits = sum(1 << p for p in ps)
            hit = once(("blocks", ref.shape, bits),
                       lambda: ((bits >> (_iota(ref.shape, 1) // B)) & 1) == 1)
            out = jnp.where(hit, v, out)
        return out

    key, lane = _iota((B, T), 0), _iota((B, T), 1)
    for n, (kb, heads) in enumerate(PASSES):
        shift = by_block([jnp.full((B, T), ((p - a) % NB - p) * B) for p, a in enumerate(heads)])
        mask[n] = jnp.where(key + kb * B <= lane + shift, 0.0, NEG)
    c_wr.wait()
    c_beta.wait()
    wrb[...] = jnp.broadcast_to(wr[...].astype(F32).reshape(1, D), (T, D)).T
    g_row = jax.nn.sigmoid(beta[...].astype(F32).reshape(1, H))
    gate[...] = jnp.broadcast_to(g_row, (T, H)).T

    background = []
    deferred = []
    later = []

    def start_background(gen):
        next(gen)
        background.append(gen)

    def pace(token):
        if background:
            try:
                background[0].send(token)
            except StopIteration:
                background.pop(0)

    def drain():
        while background:
            pace(None)

    def flush():
        while deferred:
            deferred.pop(0)()
        if later:
            later.pop(0)()

    def layernorm(s, tiles=range(NT)):
        for c in tiles:
            cols = slice(c * T, (c + 1) * T)
            mean = jnp.sum(xs[s, :, cols].astype(F32), axis=0, keepdims=True) / D
            sq = None
            for lo in range(0, D, 2 * LN_BLOCK):
                tok = yield
                cen = xs[s, lo:lo + 2 * LN_BLOCK, cols].astype(F32) - _after(mean, tok)
                part = jnp.sum((cen * cen).reshape(-1, 8, T), axis=0)
                sq = part if sq is None else sq + part
            var = jnp.sum(sq, axis=0, keepdims=True) / D
            inv = 1.0 / _round(jnp.sqrt(_round(_round(var) + EPS)))
            r = None
            for lo in range(0, D, LN_BLOCK):
                tok = yield
                rows = slice(lo, lo + LN_BLOCK)
                y = _round(xs[s, rows, cols].astype(F32) - _after(_round(mean), tok)) * inv
                y = y.astype(BF16)
                xn[s * NT + c, rows, :] = y
                part = jnp.sum((y.astype(F32) * wrb[rows, :]).reshape(-1, 8, T), axis=0)
                r = part if r is None else r + part
            rr[s, :, cols] = jnp.broadcast_to(jnp.sum(r, axis=0, keepdims=True), (8, T))

    def layernorm_now(tiles):
        start_background(layernorm(0, tiles))
        drain()

    def transpose_weights(src, dst, chunks=CHUNKS):
        for lo, hi in chunks:
            dst[lo // 2:hi // 2, :] = pltpu.bitcast(src[:, lo:hi].T, U32)

    def project(wt, rhs_of, consume, paced=0, sync=(), blocks=BLOCKS):
        for c, lo, hi in blocks:
            out = _dot(pltpu.bitcast(wt[lo // 2:hi // 2, :], BF16), rhs_of(c))
            if (c, lo) in sync:
                sync[c, lo]()
            flush()

            def post(c=c, lo=lo, hi=hi, out=out):
                consume(slice(c * T, (c + 1) * T), slice(lo, hi), out)
                for n in range(1, paced + 1):
                    row = n * (hi - lo) // paced
                    pace(out[row - 1:row])

            deferred.append(post)

    def keys(s, **kw):
        kt[s, D:, :] = jnp.zeros((_win(NG - 1) + T - D, L), BF16)

        def consume(cols, rows, k):
            kt[s, rows, cols] = k.astype(BF16)
            if s + 1 < NSEG:
                pk[s, rows, cols] = _phi(k).astype(BF16)
            if rows.stop == D and cols.stop % (2 * T) == 0:
                t0 = cols.stop - 2 * T
                for g in range(NG):
                    kg[s, g, t0 // 2:t0 // 2 + T, :] = pltpu.bitcast(
                        kt[s, _win(g):_win(g) + T, t0:t0 + 2 * T].T, U32)

        project(wkt, lambda c: xn[s * NT + c], consume, **kw)

    def queries(s, **kw):
        def consume(cols, rows, q):
            qt[s, rows.start // 2:rows.stop // 2, cols] = pltpu.bitcast(
                (q * QSCALE).astype(BF16), U32)
            if s > 0:
                pq[s, rows, cols] = _phi(q).astype(BF16)

        project(wqt, lambda c: xn[s * NT + c], consume, **kw)

    def vals(s, **kw):
        def consume(cols, rows, v):
            vt[s, rows, cols] = _round(v)

        project(wvt, lambda c: xn[s * NT + c], consume, **kw)

    mem = {}
    own = []
    for off in (0, 8):
        row = _iota((GW, GW), 0)
        col_head = _head_of(_iota((GW, GW), 1) - off)
        own.append((jnp.where(row < GF, _head_of(row), row - GF) == col_head) & (row < GF + 4))

    def remember(s):
        for g in range(NG):
            lhs = jnp.concatenate([vt[s, GF * g:GF * (g + 1), :], jnp.ones((8, L), F32)], axis=0)
            upd = _dot(lhs, pk[s, _win(g):_win(g) + GW, :], 1, 1)
            mem[g] = upd if s == 0 else mem[g] + upd
            flush()

    def recall(s):
        for g in range(NG):
            lhs = jnp.where(own[g % 2], mem[g], 0.0)
            g4 = gate[8 * (g // 2):8 * (g // 2) + 8, :]
            if g % 2:
                g4 = pltpu.roll(g4, 4, 0)
            for c in range(NT):
                cols = slice(c * T, (c + 1) * T)
                a = _dot(lhs, pq[s, _win(g):_win(g) + GW, cols])
                ot[s, GF * g:GF * (g + 1), cols] = a[0:GF] * _spread(g4 / (a[GF:GW] + 1e-6))
            flush()

    picked = []

    def route():
        tok = yield
        r = _after(_round(rr[...]), tok[:, 0:1])
        pos = (_iota(r.shape, 0) * L + _iota(r.shape, 2)).astype(F32)

        def top(scores, allowed):
            best = jnp.max(scores)
            return best, jnp.min(jnp.where((scores == best) & allowed, pos, float(S - 1)))

        r0, p0 = top(r, pos >= 0.0)
        r1, p1 = top(jnp.where(pos == p0, -jnp.inf, r), pos != p0)
        i0 = jnp.clip(p0.astype(jnp.int32), 0, S - 1)
        i1 = jnp.clip(p1.astype(jnp.int32), 0, S - 1)
        picked.extend([(r0, i0), (r1, i1)])
        for s in range(NSEG):
            ot[s, D:DE, :] = _onehot(0, i0 - s * L, (16, L)) + _onehot(1, i1 - s * L, (16, L))

    def ffn():
        (r0, i0), (r1, i1) = picked
        x_sel = (_dot(_onehot(0, i0 % T, (8, T)), xn[i0 // T], 1, 1)
                 + _dot(_onehot(1, i1 % T, (8, T)), xn[i1 // T], 1, 1))
        for _ in range(12):
            yield
        hid, y = {}, {}

        def up(i):
            both = []
            for w in (wg, wu):
                part = None
                for lo, hi in CHUNKS:
                    t = _dot(x_sel[:, lo:hi], w[lo:hi, i * T:(i + 1) * T])
                    part = t if part is None else part + t
                    yield
                both.append(part)
            hid[i] = _round(both[0] * jax.nn.sigmoid(both[0]) * both[1])

        def down(i):
            for lo, hi in CHUNKS:
                t = _dot(hid[i], wd[lo:hi, i * T:(i + 1) * T], 1, 1)
                y[lo] = t if i == 0 else y[lo] + t
                yield

        n = FF // T
        for i in range(n + 2):
            if i < n:
                yield from up(i)
            if i >= 2:
                yield from down(i - 2)
        out = jnp.concatenate([y[lo] for lo, _ in CHUNKS], axis=1)
        out = out * jax.nn.sigmoid(jnp.where(_iota((8, D), 0) == 0, r0, r1))
        wo[D:DE, :] = jnp.concatenate([out, jnp.zeros((8, D), F32)], axis=0).astype(BF16)
        transpose_weights(wo, wot)

    def q_rows(s, h, j):
        lo, w0 = DH * h, _win(h // 4)
        parts = []
        for b in range(w0, w0 + T, 16):
            if b + 16 <= lo or b >= lo + DH:
                parts.append(None)
                continue
            u = qt[s, b // 2:b // 2 + 8, j * T:(j + 1) * T]
            if not (lo <= b and b + 16 <= lo + DH):
                row = once("row", lambda: _iota((8, T), 0) * 2)
                keep = once(("rows", lo - b), lambda: (row >= lo - b) & (row < lo - b + DH))
                u = jnp.where(keep, u, jnp.zeros_like(u))
            parts.append(pltpu.roll(u, B * (h % 4), 1) if h % 4 else u)
        return parts

    def weights(parts):
        zero = once("zero", lambda: jnp.zeros((16, T), BF16))
        return jnp.concatenate(
            [zero if p is None else pltpu.bitcast(p, BF16) for p in parts], axis=0)

    mx, prob, acc, head = {}, {}, {}, {}

    def running_max(s, h, j, c, m):
        mx[s, h, j, c] = m if c == 0 else jnp.maximum(m, mx[s, h, j, c - 1])
        return mx[s, h, j, c]

    def scores(s, g, j, c):
        def k_rows(lo, n):
            return pltpu.bitcast(kg[s, g, lo // 2:(lo + n) // 2, :], BF16)

        if c < j:
            for h in range(4 * g, 4 * g + 4):
                sc = _dot(k_rows(c * T, T + B * (c + 1 == j)), weights(once((s, h, j), lambda: q_rows(s, h, j))))
                if c + 1 == j:
                    sc, head[h, j] = sc[:T], sc[T:]
                m = running_max(s, h, j, c, jnp.max(sc, axis=0, keepdims=True))
                prob[s, h, j, c] = jnp.exp2(sc - m).astype(BF16)
            return
        q = [once((s, h, j), lambda: q_rows(s, h, j)) for h in range(4 * g, 4 * g + 4)]
        sc, top = [], []
        for n, (kb, heads) in enumerate(PASSES):
            if kb == 0 and j > 0:
                sc.append(head[4 * g + n, j] + mask[n])
            else:
                parts = [None if all(q[a][i] is None for a in heads)
                         else by_block([q[a][i] for a in heads]) for i in range(T // 16)]
                sc.append(_dot(k_rows(c * T + kb * B, B), weights(parts)) + mask[n])
            top.append(jnp.max(sc[n].reshape(B // 8, 8, T), axis=0))

        def gather(a, kb, per_pass, fill):
            src = [fill] * NB
            for n, (k, heads) in enumerate(PASSES):
                for p in range(NB):
                    if k == kb and heads[p] == a:
                        src[p] = per_pass[n]
            return by_block(src)

        low = jnp.full((8, T), NEG, F32)
        m = []
        for a in range(4):
            t = gather(a, 0, top, low)
            for kb in range(1, NB):
                t = jnp.maximum(t, gather(a, kb, top, low))
            m.append(running_max(s, 4 * g + a, j, c, jnp.max(t, axis=0, keepdims=True)))
        e = [jnp.exp2(sc[n] - by_block([m[a] for a in heads]))
             for n, (_, heads) in enumerate(PASSES)]
        for a in range(4):
            prob[s, 4 * g + a, j, c] = jnp.concatenate(
                [gather(a, kb, e, None) for kb in range(NB)], axis=0).astype(BF16)

    def values(s, g, j, c):
        done = []
        for h in range(4 * g, 4 * g + 4):
            v0 = (DH * h // 8) * 8
            ones = 0 if DH * h > v0 else 23
            v = vt[s, v0:v0 + 24, c * T:(c + 1) * T]
            v = jnp.where(once(("ones", ones), lambda: _iota((24, T), 0) == ones), 1.0, v)
            o = _dot(v, prob.pop((s, h, j, c)))
            if c > 0:
                o = acc[h, j] * jnp.exp2(mx[s, h, j, c - 1] - mx[s, h, j, c]) + o
            acc[h, j] = o
            if c == j:
                o = o * ((1.0 - gate[h:h + 1, :]) / o[ones:ones + 1, :])
                done.append(pltpu.roll(o, T - B * (h % 4), 1) if h % 4 else o)
        if c == j:
            sub = _iota((8, T), 0)
            rows = [done[0][0:16]]
            for i in range(1, 4):
                rows.append(jnp.where(sub < 2 * i, done[i - 1][16:24], done[i][0:8]))
                rows.append(done[i][8:16])
            rows.append(done[3][16:24])
            o = jnp.concatenate(rows, axis=0)
            at = (s, slice(GF * g, GF * (g + 1)), slice(j * T, (j + 1) * T))
            ot[at] = o if s == 0 else ot[at] + o

    def attention(segs, hook):
        steps = [(s, g, j, c) for s in segs for g in range(NG) for j, c in TILES]
        for i in range(len(steps)):
            scores(*steps[i])
            flush()
            if i >= PV_DELAY:
                s, g, j, c = steps[i - PV_DELAY]
                values(s, g, j, c)
                hook(i - PV_DELAY, mx[s, 4 * g, j, c])
        later.extend(lambda step=step: values(*step) for step in steps[-PV_DELAY:])

    def finish(s):
        blocks, sends = BLOCKS, {(NT - 1, D): (0, D, 0, L)}
        if s == 0:
            blocks = sorted(BLOCKS, key=lambda b: b[1])
        if s == NSEG - 1:
            blocks = BLOCKS[:-1] + ((NT - 1, D - MC, D - MC // 2), (NT - 1, D - MC // 2, D))
            sends = {(NT - 2, D): (0, D, 0, L - T), (NT - 1, D - MC): (0, D - MC, L - T, L),
                     (NT - 1, D): (D - MC, D, L - T, L)}

        def consume(cols, rows, o):
            c = cols.start // T
            res = xs[s, rows, cols].astype(F32) + xn[s * NT + c, rows, :].astype(F32)
            outb[s, rows, cols] = (o + res).astype(BF16)
            if (c, rows.stop) in sends:
                send(s, *sends[c, rows.stop])

        project(wot, lambda c: ot[s, :, c * T:(c + 1) * T].astype(BF16), consume, blocks=blocks)

    x_head.wait()
    layernorm_now((0, 1))
    c_wq.start()
    c_wv.start()
    wk_head.wait()
    transpose_weights(wk, wkt, CHUNKS[:2])
    near_end = (NT - 1, MC)
    first = [(c, lo, lo + T) for c in range(NT) for lo in (0, T)]
    first += [(c, lo, lo + 160) for c in range(NT) for lo in (2 * T, 2 * T + 160)]
    keys(0, blocks=first, sync={
        (1, 0): wave([x_tail], (), lambda: layernorm_now((2, 3))),
        (NT - 1, 0): wave([wk_tail], (), lambda: transpose_weights(wk, wkt, CHUNKS[2:])),
        (NT - 1, 2 * T): wave([c_wq], x_rest, lambda: transpose_weights(wq, wqt))})
    queries(0, sync={near_end: wave([c_wv], (), lambda: transpose_weights(wv, wvt))})
    vals(0, sync={near_end: wave(x_rest, late)})
    start_background(layernorm(1))
    attention([0], lambda i, token: pace(token) if i % 10 in (0, 3, 6) else None)
    drain()
    for s in range(1, NSEG):
        more = s + 1 < NSEG
        keys(s)
        remember(s - 1)
        queries(s)
        flush()
        recall(s)
        start_background(layernorm(s + 1) if more else route())
        vals(s, paced=2, sync=() if more else {near_end: wave(late)})
        if more:
            flush()
            drain()

    routed = ffn()

    def ffn_steps(i, token):
        for _ in range(FFN_RATE[i % len(FFN_RATE)]):
            next(routed, None)

    attention(range(1, NSEG), ffn_steps)
    for _ in routed:
        pass
    for s in range(NSEG):
        finish(s)
    flush()
    for c in out_copies:
        c.wait()


@jax.jit
def pallas_parallel_sum__memory_aug_infini_attn__moe_arch_mod__prompt_kernel(
    A_x: jax.Array,
    A_wq: jax.Array,
    A_wk: jax.Array,
    A_wv: jax.Array,
    A_wo: jax.Array,
    A_beta: jax.Array,
    B_x: jax.Array,
    B_w_r: jax.Array,
    B_w_gate: jax.Array,
    B_w_up: jax.Array,
    B_w_down: jax.Array,
):
    del B_x
    scratch = [
        pltpu.VMEM((NSEG, D, L), BF16),
        pltpu.VMEM((NSEG * NT, D, T), BF16),
        pltpu.VMEM((D, D), BF16),
        pltpu.VMEM((D, D), BF16),
        pltpu.VMEM((D, D), BF16),
        pltpu.VMEM((DE, D), BF16),
        pltpu.VMEM((H,), BF16),
        pltpu.VMEM((D,), BF16),
        pltpu.VMEM((D, FF), BF16),
        pltpu.VMEM((D, FF), BF16),
        pltpu.VMEM((D, FF), BF16),
        pltpu.VMEM((D // 2, D), U32),
        pltpu.VMEM((D // 2, D), U32),
        pltpu.VMEM((D // 2, D), U32),
        pltpu.VMEM((D // 2, DE), U32),
        pltpu.VMEM((NSEG, D // 2, L), U32),
        pltpu.VMEM((NSEG, D, L), BF16),
        pltpu.VMEM((NSEG, D, L), BF16),
        pltpu.VMEM((NSEG, D, L), F32),
        pltpu.VMEM((NSEG, _win(NG - 1) + T, L), BF16),
        pltpu.VMEM((NSEG, NG, L // 2, T), U32),
        pltpu.VMEM((NSEG, DE, L), F32),
        pltpu.VMEM((NSEG, 8, L), F32),
        pltpu.VMEM((D, T), F32),
        pltpu.VMEM((H, T), F32),
        pltpu.VMEM((len(PASSES), B, T), F32),
        pltpu.VMEM((NSEG, D, L), BF16),
        pltpu.SemaphoreType.DMA((NSEG + 1,)),
        pltpu.SemaphoreType.DMA((10,)),
        pltpu.SemaphoreType.DMA((NSEG + 2,)),
    ]
    out_t = pl.pallas_call(
        _kernel,
        out_shape=jax.ShapeDtypeStruct((D, S), BF16),
        in_specs=[pl.BlockSpec(memory_space=pl.ANY)] * 10,
        out_specs=pl.BlockSpec(memory_space=pl.ANY),
        scratch_shapes=scratch,
        compiler_params=pltpu.CompilerParams(vmem_limit_bytes=100 * 1024 * 1024),
        name="infini_mod",
    )(A_x.reshape(S, D).T, A_wq, A_wk, A_wv, A_wo, A_beta, B_w_r, B_w_gate, B_w_up, B_w_down.T)
    return out_t.T.reshape(1, S, D)
```

```python
import jax
import jax.numpy as jnp
import numpy as np
from jax import lax
import jax.experimental.pallas as pl
import jax.experimental.pallas.tpu as pltpu

F32, BF16, U32 = jnp.float32, jnp.bfloat16, jnp.uint32

S, D, H, NSEG, FF = 2048, 576, 32, 4, 4608
DH = D // H
L = S // NSEG
T = 128
NT = L // T
NG = H // 4
GF = 4 * DH
GW = 80
DE = D + 16
QSCALE = float(DH ** -0.5 * np.log2(np.e))
EPS = float(np.asarray(1e-5, dtype=jnp.bfloat16))
NEG = -1e30
CHUNKS = ((0, 128), (128, 256), (256, 384), (384, 512), (512, 576))
MC = 192
BLOCKS = tuple((c, lo, lo + MC) for c in range(NT) for lo in range(0, D, MC))
LN_BLOCK = 144

TILES = ((3, 0), (0, 0), (3, 1), (3, 2), (3, 3), (1, 0), (1, 1), (2, 0), (2, 1), (2, 2))
FFN_RATE = (4, 4, 0, 4, 0, 4, 4, 0, 4, 0)
PV_DELAY = 2
NB = 4
B = T // NB
PASSES = (
    (0, (0, 0, 0, 0)), (0, (1, 1, 1, 1)), (0, (2, 2, 2, 2)), (0, (3, 3, 3, 3)),
    (1, (3, 0, 0, 0)), (1, (1, 3, 1, 1)), (1, (2, 2, 3, 2)),
    (2, (2, 2, 0, 0)), (2, (1, 3, 3, 1)),
    (3, (1, 2, 3, 0)),
)


def _dot(a, b, ca=1, cb=0):
    return lax.dot_general(a, b, (((ca,), (cb,)), ((), ())), preferred_element_type=F32)


def _iota(shape, dim):
    return lax.broadcasted_iota(jnp.int32, shape, dim)


def _round(x):
    return x.astype(BF16).astype(F32)


def _phi(t):
    return jnp.where(t > 0, t + 1.0, jnp.exp(t))


def _win(g):
    return (GF * g // 16) * 16


def _after(value, token):
    if token is None:
        return value
    return jnp.where(token * token < 0.0, 0.0, value)


def _onehot(row, lane, shape):
    return jnp.where((_iota(shape, 0) == row) & (_iota(shape, 1) == lane), 1.0, 0.0)


def _head_of(d):
    h = jnp.full(d.shape, -1, jnp.int32)
    for i in range(5):
        h = jnp.where(d >= i * DH, i, h)
    return h


def _spread(rows):
    sub = _iota(rows.shape, 0)
    full = [jnp.broadcast_to(rows[i:i + 1], rows.shape) for i in range(4)]
    out = []
    for v in range(GF // 8):
        a, b = 8 * v // DH, (8 * v + 7) // DH
        out.append(full[a] if a == b else jnp.where(sub < DH * b - 8 * v, full[a], full[b]))
    return jnp.concatenate(out, axis=0)


def _kernel(x_hbm, wq_hbm, wk_hbm, wv_hbm, wo_hbm, beta_hbm, wr_hbm, wg_hbm, wu_hbm, wd_hbm,
            out_hbm,
            xs, xn, wq, wk, wv, wo, beta, wr, wg, wu, wd,
            wqt, wkt, wvt, wot, qt, pq, pk, vt, kt, kg, ot, rr, wrb, gate, mask, outb,
            sem_x, sem_w, sem_o):
    def x_copy(s, lo, hi, sem):
        return pltpu.make_async_copy(x_hbm.at[:, pl.ds(s * L + lo, hi - lo)],
                                     xs.at[s, :, pl.ds(lo, hi - lo)], sem_x.at[sem])

    x_head, x_tail = x_copy(0, 0, L // 2, 0), x_copy(0, L // 2, L, 1)
    x_rest = [x_copy(s, 0, L, s + 1) for s in range(1, NSEG)]
    left, right = pl.ds(0, 2 * T), pl.ds(2 * T, D - 2 * T)
    c_wr, c_beta, c_wq, wk_head, wk_tail, c_wv, *late = [
        pltpu.make_async_copy(src, dst, sem_w.at[i]) for i, (src, dst) in enumerate((
            (wr_hbm, wr), (beta_hbm, beta), (wq_hbm, wq),
            (wk_hbm.at[:, left], wk.at[:, left]), (wk_hbm.at[:, right], wk.at[:, right]),
            (wv_hbm, wv),
            (wg_hbm, wg), (wu_hbm, wu), (wd_hbm, wd), (wo_hbm, wo.at[pl.ds(0, D)])))]
    out_copies = []

    def send(s, r0, r1, c0, c1):
        c = pltpu.make_async_copy(outb.at[s, pl.ds(r0, r1 - r0), pl.ds(c0, c1 - c0)],
                                  out_hbm.at[pl.ds(r0, r1 - r0), pl.ds(s * L + c0, c1 - c0)],
                                  sem_o.at[len(out_copies)])
        c.start()
        out_copies.append(c)

    def wave(wait, start=(), then=None):
        def sync():
            for c in start:
                c.start()
            for c in wait:
                c.wait()
            if then is not None:
                then()
        return sync

    for c in (c_wr, c_beta, x_head, wk_head, x_tail, wk_tail):
        c.start()

    memo = {}

    def once(name, make):
        if name not in memo:
            memo[name] = make()
        return memo[name]

    def by_block(vals):
        ref = next(v for v in vals if v is not None)
        groups = []
        for p, v in enumerate(vals):
            for got, ps in groups:
                if got is v:
                    ps.append(p)
                    break
            else:
                groups.append((v, [p]))
        groups.sort(key=lambda e: -len(e[1]))
        out = None
        for v, ps in groups:
            if v is None:
                v = once(("zero", ref.shape, ref.dtype), lambda: jnp.zeros_like(ref))
            if out is None:
                out = v
                continue
            bits = sum(1 << p for p in ps)
            hit = once(("blocks", ref.shape, bits),
                       lambda: ((bits >> (_iota(ref.shape, 1) // B)) & 1) == 1)
            out = jnp.where(hit, v, out)
        return out

    key, lane = _iota((B, T), 0), _iota((B, T), 1)
    for n, (kb, heads) in enumerate(PASSES):
        shift = by_block([jnp.full((B, T), ((p - a) % NB - p) * B) for p, a in enumerate(heads)])
        mask[n] = jnp.where(key + kb * B <= lane + shift, 0.0, NEG)
    c_wr.wait()
    c_beta.wait()
    wrb[...] = jnp.broadcast_to(wr[...].astype(F32).reshape(1, D), (T, D)).T
    g_row = jax.nn.sigmoid(beta[...].astype(F32).reshape(1, H))
    gate[...] = jnp.broadcast_to(g_row, (T, H)).T

    background = []
    deferred = []
    later = []

    def start_background(gen):
        next(gen)
        background.append(gen)

    def pace(token):
        if background:
            try:
                background[0].send(token)
            except StopIteration:
                background.pop(0)

    def drain():
        while background:
            pace(None)

    def flush():
        while deferred:
            deferred.pop(0)()
        if later:
            later.pop(0)()

    def layernorm(s, tiles=range(NT)):
        for c in tiles:
            cols = slice(c * T, (c + 1) * T)
            mean = jnp.sum(xs[s, :, cols].astype(F32), axis=0, keepdims=True) / D
            sq = None
            for lo in range(0, D, 2 * LN_BLOCK):
                tok = yield
                cen = xs[s, lo:lo + 2 * LN_BLOCK, cols].astype(F32) - _after(mean, tok)
                part = jnp.sum((cen * cen).reshape(-1, 8, T), axis=0)
                sq = part if sq is None else sq + part
            var = jnp.sum(sq, axis=0, keepdims=True) / D
            inv = 1.0 / _round(jnp.sqrt(_round(_round(var) + EPS)))
            for lo in range(0, D, LN_BLOCK):
                tok = yield
                rows = slice(lo, lo + LN_BLOCK)
                y = _round(xs[s, rows, cols].astype(F32) - _after(_round(mean), tok)) * inv
                xn[s * NT + c, rows, :] = y.astype(BF16)

    def layernorm_now(tiles):
        start_background(layernorm(0, tiles))
        drain()

    def transpose_weights(src, dst, chunks=CHUNKS):
        for lo, hi in chunks:
            dst[lo // 2:hi // 2, :] = pltpu.bitcast(src[:, lo:hi].T, U32)

    def project(wt, rhs_of, consume, paced=0, sync=(), blocks=BLOCKS):
        for c, lo, hi in blocks:
            out = _dot(pltpu.bitcast(wt[lo // 2:hi // 2, :], BF16), rhs_of(c))
            if (c, lo) in sync:
                sync[c, lo]()
            flush()

            def post(c=c, lo=lo, hi=hi, out=out):
                consume(slice(c * T, (c + 1) * T), slice(lo, hi), out)
                for n in range(1, paced + 1):
                    row = n * (hi - lo) // paced
                    pace(out[row - 1:row])

            deferred.append(post)

    def keys(s, **kw):
        kt[s, D:, :] = jnp.zeros((_win(NG - 1) + T - D, L), BF16)

        def consume(cols, rows, k):
            kt[s, rows, cols] = k.astype(BF16)
            if s + 1 < NSEG:
                pk[s, rows, cols] = _phi(k).astype(BF16)
            if rows.stop == D and cols.stop % (2 * T) == 0:
                t0 = cols.stop - 2 * T
                for g in range(NG):
                    kg[s, g, t0 // 2:t0 // 2 + T, :] = pltpu.bitcast(
                        kt[s, _win(g):_win(g) + T, t0:t0 + 2 * T].T, U32)

        project(wkt, lambda c: xn[s * NT + c], consume, **kw)

    def queries(s, **kw):
        def consume(cols, rows, q):
            qt[s, rows.start // 2:rows.stop // 2, cols] = pltpu.bitcast(
                (q * QSCALE).astype(BF16), U32)
            if s > 0:
                pq[s, rows, cols] = _phi(q).astype(BF16)

        project(wqt, lambda c: xn[s * NT + c], consume, **kw)

    def vals(s, **kw):
        def consume(cols, rows, v):
            vt[s, rows, cols] = _round(v)

        project(wvt, lambda c: xn[s * NT + c], consume, **kw)

    mem = {}
    own = []
    for off in (0, 8):
        row = _iota((GW, GW), 0)
        col_head = _head_of(_iota((GW, GW), 1) - off)
        own.append((jnp.where(row < GF, _head_of(row), row - GF) == col_head) & (row < GF + 4))

    def remember(s):
        for g in range(NG):
            lhs = jnp.concatenate([vt[s, GF * g:GF * (g + 1), :], jnp.ones((8, L), F32)], axis=0)
            upd = _dot(lhs, pk[s, _win(g):_win(g) + GW, :], 1, 1)
            mem[g] = upd if s == 0 else mem[g] + upd
            flush()

    def recall(s):
        for g in range(NG):
            lhs = jnp.where(own[g % 2], mem[g], 0.0)
            g4 = gate[8 * (g // 2):8 * (g // 2) + 8, :]
            if g % 2:
                g4 = pltpu.roll(g4, 4, 0)
            for c in range(NT):
                cols = slice(c * T, (c + 1) * T)
                a = _dot(lhs, pq[s, _win(g):_win(g) + GW, cols])
                ot[s, GF * g:GF * (g + 1), cols] = a[0:GF] * _spread(g4 / (a[GF:GW] + 1e-6))
            flush()

    picked = []

    def router_scores(s):
        for c in range(NT):
            tok = yield
            r = jnp.sum((xn[s * NT + c].astype(F32) * wrb[...]).reshape(-1, 8, T), axis=0)
            r = jnp.sum(_after(r, tok), axis=0, keepdims=True)
            rr[s, :, c * T:(c + 1) * T] = jnp.broadcast_to(r, (8, T))

    def route():
        tok = yield
        r = _after(_round(rr[...]), tok[:, 0:1])
        pos = (_iota(r.shape, 0) * L + _iota(r.shape, 2)).astype(F32)

        def top(scores, allowed):
            best = jnp.max(scores)
            return best, jnp.min(jnp.where((scores == best) & allowed, pos, float(S - 1)))

        r0, p0 = top(r, pos >= 0.0)
        r1, p1 = top(jnp.where(pos == p0, -jnp.inf, r), pos != p0)
        i0 = jnp.clip(p0.astype(jnp.int32), 0, S - 1)
        i1 = jnp.clip(p1.astype(jnp.int32), 0, S - 1)
        picked.extend([(r0, i0), (r1, i1)])
        for s in range(NSEG):
            ot[s, D:DE, :] = _onehot(0, i0 - s * L, (16, L)) + _onehot(1, i1 - s * L, (16, L))

    def ffn():
        (r0, i0), (r1, i1) = picked
        x_sel = (_dot(_onehot(0, i0 % T, (8, T)), xn[i0 // T], 1, 1)
                 + _dot(_onehot(1, i1 % T, (8, T)), xn[i1 // T], 1, 1))
        for _ in range(12):
            yield
        hid, y = {}, {}

        def up(i):
            both = []
            for w in (wg, wu):
                part = None
                for lo, hi in CHUNKS:
                    t = _dot(x_sel[:, lo:hi], w[lo:hi, i * T:(i + 1) * T])
                    part = t if part is None else part + t
                    yield
                both.append(part)
            hid[i] = _round(both[0] * jax.nn.sigmoid(both[0]) * both[1])

        def down(i):
            for lo, hi in CHUNKS:
                t = _dot(hid[i], wd[lo:hi, i * T:(i + 1) * T], 1, 1)
                y[lo] = t if i == 0 else y[lo] + t
                yield

        n = FF // T
        for i in range(n + 2):
            if i < n:
                yield from up(i)
            if i >= 2:
                yield from down(i - 2)
        out = jnp.concatenate([y[lo] for lo, _ in CHUNKS], axis=1)
        out = out * jax.nn.sigmoid(jnp.where(_iota((8, D), 0) == 0, r0, r1))
        wo[D:DE, :] = jnp.concatenate([out, jnp.zeros((8, D), F32)], axis=0).astype(BF16)
        transpose_weights(wo, wot)

    def q_rows(s, h, j):
        lo, w0 = DH * h, _win(h // 4)
        parts = []
        for b in range(w0, w0 + T, 16):
            if b + 16 <= lo or b >= lo + DH:
                parts.append(None)
                continue
            u = qt[s, b // 2:b // 2 + 8, j * T:(j + 1) * T]
            if not (lo <= b and b + 16 <= lo + DH):
                row = once("row", lambda: _iota((8, T), 0) * 2)
                keep = once(("rows", lo - b), lambda: (row >= lo - b) & (row < lo - b + DH))
                u = jnp.where(keep, u, jnp.zeros_like(u))
            parts.append(pltpu.roll(u, B * (h % 4), 1) if h % 4 else u)
        return parts

    def weights(parts):
        zero = once("zero", lambda: jnp.zeros((16, T), BF16))
        return jnp.concatenate(
            [zero if p is None else pltpu.bitcast(p, BF16) for p in parts], axis=0)

    mx, prob, acc, head = {}, {}, {}, {}

    def running_max(s, h, j, c, m):
        mx[s, h, j, c] = m if c == 0 else jnp.maximum(m, mx[s, h, j, c - 1])
        return mx[s, h, j, c]

    def scores(s, g, j, c):
        def k_rows(lo, n):
            return pltpu.bitcast(kg[s, g, lo // 2:(lo + n) // 2, :], BF16)

        if c < j:
            for h in range(4 * g, 4 * g + 4):
                sc = _dot(k_rows(c * T, T + B * (c + 1 == j)), weights(once((s, h, j), lambda: q_rows(s, h, j))))
                if c + 1 == j:
                    sc, head[h, j] = sc[:T], sc[T:]
                m = running_max(s, h, j, c, jnp.max(sc, axis=0, keepdims=True))
                prob[s, h, j, c] = jnp.exp2(sc - m).astype(BF16)
            return
        q = [once((s, h, j), lambda: q_rows(s, h, j)) for h in range(4 * g, 4 * g + 4)]
        sc, top = [], []
        for n, (kb, heads) in enumerate(PASSES):
            if kb == 0 and j > 0:
                sc.append(head[4 * g + n, j] + mask[n])
            else:
                parts = [None if all(q[a][i] is None for a in heads)
                         else by_block([q[a][i] for a in heads]) for i in range(T // 16)]
                sc.append(_dot(k_rows(c * T + kb * B, B), weights(parts)) + mask[n])
            top.append(jnp.max(sc[n].reshape(B // 8, 8, T), axis=0))

        def gather(a, kb, per_pass, fill):
            src = [fill] * NB
            for n, (k, heads) in enumerate(PASSES):
                for p in range(NB):
                    if k == kb and heads[p] == a:
                        src[p] = per_pass[n]
            return by_block(src)

        m = []
        for a in range(4):
            t = top[a]
            for kb in range(1, NB):
                t = jnp.maximum(t, gather(a, kb, top, t))
            m.append(running_max(s, 4 * g + a, j, c, jnp.max(t, axis=0, keepdims=True)))
        e = [jnp.exp2(sc[n] - by_block([m[a] for a in heads]))
             for n, (_, heads) in enumerate(PASSES)]
        for a in range(4):
            prob[s, 4 * g + a, j, c] = jnp.concatenate(
                [gather(a, kb, e, None) for kb in range(NB)], axis=0).astype(BF16)

    def values(s, g, j, c):
        done = []
        for h in range(4 * g, 4 * g + 4):
            v0 = (DH * h // 8) * 8
            ones = 0 if DH * h > v0 else 23
            v = vt[s, v0:v0 + 24, c * T:(c + 1) * T]
            v = jnp.where(once(("ones", ones), lambda: _iota((24, T), 0) == ones), 1.0, v)
            o = _dot(v, prob.pop((s, h, j, c)))
            if c > 0:
                o = acc[h, j] * jnp.exp2(mx[s, h, j, c - 1] - mx[s, h, j, c]) + o
            acc[h, j] = o
            if c == j:
                o = o * ((1.0 - gate[h:h + 1, :]) / o[ones:ones + 1, :])
                done.append(pltpu.roll(o, T - B * (h % 4), 1) if h % 4 else o)
        if c == j:
            sub = _iota((8, T), 0)
            rows = [done[0][0:16]]
            for i in range(1, 4):
                rows.append(jnp.where(sub < 2 * i, done[i - 1][16:24], done[i][0:8]))
                rows.append(done[i][8:16])
            rows.append(done[3][16:24])
            o = jnp.concatenate(rows, axis=0)
            at = (s, slice(GF * g, GF * (g + 1)), slice(j * T, (j + 1) * T))
            ot[at] = o if s == 0 else ot[at] + o

    def attention(segs, hook):
        steps = [(s, g, j, c) for s in segs for g in range(NG) for j, c in TILES]
        for i in range(len(steps)):
            scores(*steps[i])
            flush()
            if i >= PV_DELAY:
                s, g, j, c = steps[i - PV_DELAY]
                values(s, g, j, c)
                hook(i - PV_DELAY, mx[s, 4 * g, j, c])
        later.extend(lambda step=step: values(*step) for step in steps[-PV_DELAY:])

    def finish(s):
        blocks, sends = BLOCKS, {(NT - 1, D): (0, D, 0, L)}
        if s == 0:
            blocks = sorted(BLOCKS, key=lambda b: b[1])
        if s == NSEG - 1:
            blocks = BLOCKS[:-1] + ((NT - 1, D - MC, D - MC // 2), (NT - 1, D - MC // 2, D))
            sends = {(NT - 2, D): (0, D, 0, L - T), (NT - 1, D - MC): (0, D - MC, L - T, L),
                     (NT - 1, D): (D - MC, D, L - T, L)}

        def consume(cols, rows, o):
            c = cols.start // T
            res = xs[s, rows, cols].astype(F32) + xn[s * NT + c, rows, :].astype(F32)
            outb[s, rows, cols] = (o + res).astype(BF16)
            if (c, rows.stop) in sends:
                send(s, *sends[c, rows.stop])

        project(wot, lambda c: ot[s, :, c * T:(c + 1) * T].astype(BF16), consume, blocks=blocks)

    x_head.wait()
    layernorm_now((0, 1))
    c_wq.start()
    c_wv.start()
    wk_head.wait()
    transpose_weights(wk, wkt, CHUNKS[:2])
    near_end = (NT - 1, MC)
    first = [(c, lo, lo + T) for c in range(NT) for lo in (0, T)]
    first += [(c, lo, lo + 160) for c in range(NT) for lo in (2 * T, 2 * T + 160)]
    keys(0, blocks=first, sync={
        (1, 0): wave([x_tail], (), lambda: layernorm_now((2, 3))),
        (NT - 1, 0): wave([wk_tail], (), lambda: transpose_weights(wk, wkt, CHUNKS[2:])),
        (NT - 1, 2 * T): wave([c_wq], x_rest, lambda: transpose_weights(wq, wqt))})
    start_background(router_scores(0))
    queries(0, paced=1, sync={near_end: wave([c_wv], (), lambda: transpose_weights(wv, wvt))})
    vals(0, sync={near_end: wave(x_rest, late)})
    start_background(layernorm(1))
    attention([0], lambda i, token: pace(token) if i % 10 in (0, 3, 6) else None)
    drain()
    for s in range(1, NSEG):
        more = s + 1 < NSEG
        keys(s)
        remember(s - 1)
        start_background(router_scores(s))
        queries(s, paced=1)
        flush()
        recall(s)
        start_background(layernorm(s + 1) if more else route())
        vals(s, paced=3, sync=() if more else {near_end: wave(late)})

    routed = ffn()

    def ffn_steps(i, token):
        for _ in range(FFN_RATE[i % len(FFN_RATE)]):
            next(routed, None)

    attention(range(1, NSEG), ffn_steps)
    for _ in routed:
        pass
    for s in range(NSEG):
        finish(s)
    flush()
    for c in out_copies:
        c.wait()


@jax.jit
def pallas_parallel_sum__memory_aug_infini_attn__moe_arch_mod__prompt_kernel(
    A_x: jax.Array,
    A_wq: jax.Array,
    A_wk: jax.Array,
    A_wv: jax.Array,
    A_wo: jax.Array,
    A_beta: jax.Array,
    B_x: jax.Array,
    B_w_r: jax.Array,
    B_w_gate: jax.Array,
    B_w_up: jax.Array,
    B_w_down: jax.Array,
):
    del B_x
    scratch = [
        pltpu.VMEM((NSEG, D, L), BF16),
        pltpu.VMEM((NSEG * NT, D, T), BF16),
        pltpu.VMEM((D, D), BF16),
        pltpu.VMEM((D, D), BF16),
        pltpu.VMEM((D, D), BF16),
        pltpu.VMEM((DE, D), BF16),
        pltpu.VMEM((H,), BF16),
        pltpu.VMEM((D,), BF16),
        pltpu.VMEM((D, FF), BF16),
        pltpu.VMEM((D, FF), BF16),
        pltpu.VMEM((D, FF), BF16),
        pltpu.VMEM((D // 2, D), U32),
        pltpu.VMEM((D // 2, D), U32),
        pltpu.VMEM((D // 2, D), U32),
        pltpu.VMEM((D // 2, DE), U32),
        pltpu.VMEM((NSEG, D // 2, L), U32),
        pltpu.VMEM((NSEG, D, L), BF16),
        pltpu.VMEM((NSEG, D, L), BF16),
        pltpu.VMEM((NSEG, D, L), F32),
        pltpu.VMEM((NSEG, _win(NG - 1) + T, L), BF16),
        pltpu.VMEM((NSEG, NG, L // 2, T), U32),
        pltpu.VMEM((NSEG, DE, L), F32),
        pltpu.VMEM((NSEG, 8, L), F32),
        pltpu.VMEM((D, T), F32),
        pltpu.VMEM((H, T), F32),
        pltpu.VMEM((len(PASSES), B, T), F32),
        pltpu.VMEM((NSEG, D, L), BF16),
        pltpu.SemaphoreType.DMA((NSEG + 1,)),
        pltpu.SemaphoreType.DMA((10,)),
        pltpu.SemaphoreType.DMA((NSEG + 2,)),
    ]
    out_t = pl.pallas_call(
        _kernel,
        out_shape=jax.ShapeDtypeStruct((D, S), BF16),
        in_specs=[pl.BlockSpec(memory_space=pl.ANY)] * 10,
        out_specs=pl.BlockSpec(memory_space=pl.ANY),
        scratch_shapes=scratch,
        compiler_params=pltpu.CompilerParams(vmem_limit_bytes=100 * 1024 * 1024),
        name="infini_mod",
    )(A_x.reshape(S, D).T, A_wq, A_wk, A_wv, A_wo, A_beta, B_w_r, B_w_gate, B_w_up, B_w_down.T)
    return out_t.T.reshape(1, S, D)
```
